```python
import jax
import jax.numpy as jnp

def _softmax(x, axis=-1):
    return jax.nn.softmax(x, axis=axis)

def _gelu(x):
    return jax.nn.gelu(x, approximate=True)

def _silu(x):
    return jax.nn.silu(x)

def _sigmoid(x):
    return jax.nn.sigmoid(x)

def _layernorm(x, axis=-1, eps=1e-05):
    m = jnp.mean(x, axis=axis, keepdims=True)
    v = jnp.var(x, axis=axis, keepdims=True)
    return (x - m) / jnp.sqrt(v + eps)

def _scatter_add(tgt, idx, src, axis=0):
    return tgt.at[idx].add(src)

def _segment_sum(src, seg, n):
    return jax.ops.segment_sum(src, seg, n)

class _Rng:

    def __init__(self, key):
        self._k = key

    def _next(self):
        self._k, sub = jax.random.split(self._k)
        return sub

    def normal(self, shape):
        return jax.random.normal(self._next(), shape, dtype=jnp.bfloat16)

    def randint(self, lo, hi, shape):
        return jax.random.randint(self._next(), shape, lo, hi, dtype=jnp.int32)

    def uniform(self, shape, lo=0.0, hi=1.0):
        return jax.random.uniform(self._next(), shape, jnp.bfloat16, lo, hi)

    def permutation(self, n):
        return jax.random.permutation(self._next(), n)
kernel_name = 'sequential_preLN__ssm_conv_s4__mixer_gmlp__prompt'

def _fwd_setup_inputs():
    _rng = _Rng(jax.random.key(int.from_bytes(__import__("os").urandom(4), "little")))
    _w = lambda a: (lambda t: t.astype(jnp.bfloat16) if jnp.issubdtype(t.dtype, jnp.floating) else t)(jnp.asarray(a))

    def _A_setup():
        B, L, D, N = (1, 2048, 576, 128)
        A_re = -jnp.exp((lambda *s: _rng.normal(s) * 0.05)(D, N))
        A_im = jnp.pi * (lambda *s: _rng.normal(s) * 0.05)(D, N)
        B_re = (lambda *s: _rng.normal(s) * 0.05)(D, N)
        B_im = (lambda *s: _rng.normal(s) * 0.05)(D, N)
        C_re = (lambda *s: _rng.normal(s) * 0.05)(D, N)
        C_im = (lambda *s: _rng.normal(s) * 0.05)(D, N)
        log_dt = (lambda *s: _rng.normal(s) * 0.05)(D) * 0.5 - 4.0
        Dskip = (lambda *s: _rng.normal(s) * 0.05)(D)
        return {'u': _w((lambda *s: _rng.normal(s) * 0.05)(B, L, D)), 'A_re': _w(A_re), 'A_im': _w(A_im), 'B_re': _w(B_re), 'B_im': _w(B_im), 'C_re': _w(C_re), 'C_im': _w(C_im), 'log_dt': _w(log_dt), 'Dskip': _w(Dskip)}
    _A_in = _A_setup()

    def _B_setup():
        B, S, D, F = (1, 2048, 576, 4608)
        Fh = F // 2
        return {'x': _w((lambda *s: _rng.normal(s) * 0.05)(B, S, D)), 'w_in': _w((lambda *s: _rng.normal(s) * 0.05)(D, 2 * Fh)), 'w_sp': _w(0.01 * (lambda *s: _rng.normal(s) * 0.05)(S, S)), 'b_sp': _w(1.0 + 0.01 * (lambda *s: _rng.normal(s) * 0.05)(S)), 'w_out': _w((lambda *s: _rng.normal(s) * 0.05)(Fh, D))}
    _B_in = _B_setup()
    return {'A_u': _A_in['u'], 'A_A_re': _A_in['A_re'], 'A_A_im': _A_in['A_im'], 'A_B_re': _A_in['B_re'], 'A_B_im': _A_in['B_im'], 'A_C_re': _A_in['C_re'], 'A_C_im': _A_in['C_im'], 'A_log_dt': _A_in['log_dt'], 'A_Dskip': _A_in['Dskip'], 'B_x': _B_in['x'], 'B_w_in': _B_in['w_in'], 'B_w_sp': _B_in['w_sp'], 'B_b_sp': _B_in['b_sp'], 'B_w_out': _B_in['w_out']}

def _fwd_reference(A_u, A_A_re, A_A_im, A_B_re, A_B_im, A_C_re, A_C_im, A_log_dt, A_Dskip, B_x, B_w_in, B_w_sp, B_b_sp, B_w_out):

    def _A_ref(u, A_re, A_im, B_re, B_im, C_re, C_im, log_dt, Dskip):
        Bsz, L, D = u.shape
        dt = jnp.exp(log_dt)[:, None]
        A = A_re + 1j * A_im
        Bc = B_re + 1j * B_im
        Cc = C_re + 1j * C_im
        logdA = dt * A
        dB = dt * Bc
        l = (lambda x, dt: x.astype(dt))(jnp.arange(L), A_re.dtype)
        P = jnp.exp(logdA[:, :, None] * l[None, None, :])
        K = jnp.einsum('dn,dnl,dn->dl', Cc, P, dB).real
        L2 = 2 * L
        Kp = jnp.pad(K, ((0, 0), (0, L)))
        up = (lambda x, *d: x.transpose(*d))(u, 0, 2, 1)
        up = jnp.pad(up, ((0, 0), (0, 0), (0, L)))
        Kf = (lambda x, axes=(-2, -1): jnp.fft.rfft2(x.astype(jnp.float32), axes=axes))(Kp[:, None, :], axes=(-2, -1))
        Uf = (lambda x, axes=(-2, -1): jnp.fft.rfft2(x.astype(jnp.float32), axes=axes))(up[:, :, None, :], axes=(-2, -1))
        Yf = Uf * Kf[None, :, :, :]
        y = (lambda x, s, axes=(-2, -1): jnp.fft.irfft2(x, s=s, axes=axes).astype(jnp.bfloat16))(Yf, (1, L2), axes=(-2, -1))[:, :, 0, :L]
        y = (lambda x, *d: x.transpose(*d))(y, 0, 2, 1) + u * Dskip[None, None, :]
        return y

    def _B_ref(x, w_in, w_sp, b_sp, w_out):
        B, S, D = x.shape
        F = w_in.shape[-1]
        Fh = F // 2
        z = _gelu(jnp.einsum('bsd,df->bsf', x, w_in))
        z1 = z[..., :Fh].copy()
        z2 = _layernorm(z[..., Fh:], axis=-1)
        g = jnp.einsum('ts,bsf->btf', w_sp, z2) + b_sp[None, :, None]
        return jnp.einsum('bsf,fd->bsd', z1 * g, w_out)
    x = A_u
    h = x + _A_ref(_layernorm(x, axis=-1), A_A_re, A_A_im, A_B_re, A_B_im, A_C_re, A_C_im, A_log_dt, A_Dskip)
    h2 = h + _B_ref(_layernorm(h, axis=-1), B_w_in, B_w_sp, B_b_sp, B_w_out)
    return h2

def setup_inputs():
    _inp = _fwd_setup_inputs()
    _gk = jax.random.fold_in(jax.random.key(int.from_bytes(__import__("os").urandom(4), "little")), 2 ** 31 - 1)
    _shapes = [[1, 2048, 576]]
    _dtypes = ['bfloat16']
    _gks = jax.random.split(_gk, len(_shapes))
    _gs = [jax.random.normal(k, s, dtype=jnp.dtype(d)) * 0.05 for k, s, d in zip(_gks, _shapes, _dtypes)]
    _inp['grad_out'] = _gs[0]
    return _inp

def reference(A_u, A_A_re, A_A_im, A_B_re, A_B_im, A_C_re, A_C_im, A_log_dt, A_Dskip, B_w_in, B_w_sp, B_b_sp, B_w_out, B_x, grad_out):
    _const = dict(B_x=B_x)

    def _f(*_d):
        return _fwd_reference(**{'A_u': _d[0], 'A_A_re': _d[1], 'A_A_im': _d[2], 'A_B_re': _d[3], 'A_B_im': _d[4], 'A_C_re': _d[5], 'A_C_im': _d[6], 'A_log_dt': _d[7], 'A_Dskip': _d[8], 'B_w_in': _d[9], 'B_w_sp': _d[10], 'B_b_sp': _d[11], 'B_w_out': _d[12], **_const})
    _out, _vjp = jax.vjp(_f, A_u, A_A_re, A_A_im, A_B_re, A_B_im, A_C_re, A_C_im, A_log_dt, A_Dskip, B_w_in, B_w_sp, B_b_sp, B_w_out)
    _grads = _vjp(grad_out)
    _out0 = jnp.asarray(_out)
    return (_out0, *[jnp.asarray(_g) for _g in _grads])
```

```python
import functools
import numpy as np
import jax
import jax.numpy as jnp
from jax import lax
import jax.experimental.pallas as pl
import jax.experimental.pallas.tpu as pltpu

bf = jnp.bfloat16
f32 = jnp.float32
L = 2048
D = 576
N = 128
T = 128
NC = 16
FH = 2304
EPS = 1e-5
C0 = float(np.sqrt(2.0 / np.pi))
C1 = 0.044715 * C0

NN = (((1,), (0,)), ((), ()))
NT = (((1,), (1,)), ((), ()))
TN = (((0,), (0,)), ((), ()))


def _bf16_round_np(a):
    a = np.ascontiguousarray(np.asarray(a, dtype=np.float32))
    u = a.view(np.uint32).astype(np.uint64)
    r = ((u + 0x7FFF + ((u >> 16) & 1)) >> 16) << 16
    return r.astype(np.uint32).view(np.float32)


def _build_consts():
    lt = _bf16_round_np(np.arange(L)).astype(np.int64)
    bases = []
    for m in range(16):
        step = 1 if m < 2 else 2 if m < 4 else 4 if m < 8 else 8
        for a in range(0, 8, step):
            bases.append(128 * m + a)
    bases.append(2048)
    pos = {}
    valid = set(lt.tolist())
    for i, bs in enumerate(bases):
        t, slot = divmod(i, 8)
        for b in range(16):
            v = bs + 8 * b
            if v in valid:
                assert v not in pos
                pos[v] = (t, 8 * ((b + 1) % 16) + slot)
    assert set(pos.keys()) == valid
    theta = np.pi * (2 * np.arange(T) + 1) / (2 * T)
    tau = np.arange(T)
    Fm = np.concatenate([np.cos(np.outer(tau, theta)), -np.sin(np.outer(tau, theta))], 1)
    Mp = {}
    for m in range(16):
        for l in range(max(0, 128 * m - 127), min(L, 128 * m + 128)):
            r = l - 128 * m
            t, ln = pos[int(lt[l])]
            M = Mp.setdefault((m, t), np.zeros((128, 256)))
            M[ln, :128] += np.cos(theta * r) / T
            M[ln, 128:] += -np.sin(theta * r) / T
    keys = sorted(Mp.keys())
    Mcat = np.concatenate([Mp[k] for k in keys], 0)
    return bases, keys, Mcat.astype(np.float32), Fm.astype(np.float32)


BASES, MKEYS, MCAT_NP, F_NP = _build_consts()
NB = len(BASES)
MIDX = {k: i for i, k in enumerate(MKEYS)}


def _dot(a, b, dims=NN):
    return lax.dot_general(a, b, dims, preferred_element_type=f32)


def _cmul(ar, ai, br, bi):
    return ar * br - ai * bi, ar * bi + ai * br


def _csq(ar, ai):
    return ar * ar - ai * ai, 2.0 * ar * ai


def _gelu_both(x):
    x2 = x * x
    u = x * (C0 + C1 * x2)
    th = jnp.tanh(u)
    hx = 0.5 * x
    s = 1.0 + th
    return hx * s, 0.5 * s + hx * (1.0 - th * th) * (C0 + (3.0 * C1) * x2)


def _ln0(x):
    m = jnp.sum(x, axis=0, keepdims=True) * (1.0 / D)
    xc = x - m
    v = jnp.sum(xc * xc, axis=0, keepdims=True) * (1.0 / D)
    r = lax.rsqrt(v + EPS)
    return xc * r, r


def _loop(name, n, body):
    with jax.named_scope(name):
        lax.fori_loop(0, n, body, 0)


def _steps(m):
    return 1 if m < 2 else 2 if m < 4 else 4 if m < 8 else 8


def kernel(u_hbm, do_hbm, win_hbm, wsp_hbm, wout_hbm, m_hbm,
           Ar_ref, Ai_ref, Br_ref, Bi_ref, Cr_ref, Ci_ref, logdt_ref, dsk_ref, bsp_ref, F_ref,
           h2_hbm, du_hbm, dAr_ref, dAi_ref, dBr_ref, dBi_ref, dCr_ref, dCi_ref, dlog_ref, dD_ref,
           dwin_hbm, dwsp_hbm, dbsp_ref, dwout_hbm,
           U, DO, WIN, WSP, WOUTT, MM, XNT, HT, HNT, HN, DOT_, DHT,
           Z1, Z2N, DG, Q1, GD2, XH, KH, PAR, DTC, DSC, BCOL, RS1, RS2, DBROW, sem_in, sem_out):
    def cin(src, dst, i):
        return pltpu.make_async_copy(src, dst, sem_in.at[i])

    DUT = HT
    cp_u = cin(u_hbm, U, 0)
    cp_m = cin(m_hbm, MM, 1)
    cp_do = cin(do_hbm, DOT_, 2)
    cp_wout = cin(wout_hbm, WOUTT, 3)
    cp_win = cin(win_hbm, WIN, 4)
    cp_wsp = cin(wsp_hbm, WSP, 5)
    for c in (cp_u, cp_m, cp_do, cp_wout, cp_win, cp_wsp):
        c.start()

    Fm = F_ref[...]

    dt_row = jnp.exp(logdt_ref[...].astype(f32)[None, :]).astype(bf).astype(f32)
    DTC[...] = jnp.broadcast_to(dt_row, (128, D)).T
    DSC[...] = jnp.broadcast_to(dsk_ref[...].astype(f32)[None, :], (128, D)).T
    bsp_row = bsp_ref[...].astype(f32)[None, :]
    for i in range(16):
        BCOL[i * 128:(i + 1) * 128, :] = jnp.broadcast_to(
            bsp_row[:, i * 128:(i + 1) * 128], (128, 128)).T

    def s0(i, c):
        r = pl.ds(pl.multiple_of(i * 64, 64), 64)
        dt = DTC[r, :]
        ar = dt * Ar_ref[r, :].astype(f32)
        ai = dt * Ai_ref[r, :].astype(f32)
        cbr, cbi = _cmul(Cr_ref[r, :].astype(f32), Ci_ref[r, :].astype(f32),
                         Br_ref[r, :].astype(f32), Bi_ref[r, :].astype(f32))
        PAR[0, r, :] = dt * cbr
        PAR[1, r, :] = dt * cbi
        e = jnp.exp(ar)
        l1 = (e * jnp.cos(ai), e * jnp.sin(ai))
        l2 = _csq(*l1)
        l4 = _csq(*l2)
        l8 = _csq(*l4)
        l128 = _csq(*_csq(*_csq(*_csq(*l8))))
        for k, z in enumerate((l1, l2, l4, l128, l8)):
            PAR[2 + 2 * k, r, :] = z[0]
            PAR[3 + 2 * k, r, :] = z[1]
        return c
    _loop("s0", 9, s0)
    for c in range(8):
        PAR[12, pl.ds(c, 72, stride=8), :] = PAR[10, pl.ds(7 - c, 72, stride=8), :]
        PAR[13, pl.ds(c, 72, stride=8), :] = -PAR[11, pl.ds(7 - c, 72, stride=8), :]

    lane = lax.broadcasted_iota(jnp.int32, (8, 128), 1)
    subl = lax.broadcasted_iota(jnp.int32, (8, 128), 0)
    slot_mask = [(lane & 7) == s for s in range(8)]
    diag_mask = (lane & 7) == subl
    lane8 = ((lane >> 3) * 8).astype(f32)

    def ssm_fwd(KC, YH):
        def s1_group(g):
            r = pl.ds(pl.multiple_of(g * 8, 8), 8)
            l8 = (PAR[12, r, :], PAR[13, r, :])
            E = [(jnp.ones((8, 128), f32), jnp.zeros((8, 128), f32)), l8]
            for b in range(2, 16):
                E.append(_cmul(*E[-1], *l8))
            rhs = jnp.concatenate(
                [jnp.concatenate([e[0] for e in E], axis=0).astype(bf),
                 jnp.concatenate([e[1] for e in E], axis=0).astype(bf)], axis=1)
            lam = {1: (PAR[2, r, :], PAR[3, r, :]), 2: (PAR[4, r, :], PAR[5, r, :]),
                   4: (PAR[6, r, :], PAR[7, r, :])}
            l128 = (PAR[8, r, :], PAR[9, r, :])
            cur = (PAR[0, r, :], PAR[1, r, :])
            Us = []
            for m in range(17):
                z = cur
                if m < 16:
                    st = _steps(m)
                    for a in range(0, 8, st):
                        Us.append(z)
                        if a + st < 8:
                            z = _cmul(*z, *lam[st])
                else:
                    Us.append(z)
                if m < 16:
                    cur = _cmul(*cur, *l128)
            zero = jnp.zeros((8, 128), f32)
            lhs = jnp.concatenate(
                [jnp.concatenate([x[0] for x in Us] + [zero], axis=0).astype(bf),
                 jnp.concatenate([x[1] for x in Us] + [zero], axis=0).astype(bf)], axis=1)
            out = _dot(lhs, rhs, NT)
            for t in range(6):
                acc = None
                for slot in range(8):
                    i = 8 * t + slot
                    if i >= NB:
                        break
                    rr = pltpu.roll(out[8 * i:8 * i + 8, :], slot + 1, 1, stride=1, stride_axis=0)
                    acc = jnp.where(slot_mask[slot], rr, 0.0 if acc is None else acc)
                KC[r, t * 128:(t + 1) * 128] = acc

        def s1(i, c):
            s1_group(2 * i)
            s1_group(2 * i + 1)
            return c
        _loop("s1", 36, s1)

        cp_m.wait()
        for m in range(16):
            ts = [t for (mm, t) in MKEYS if mm == m]
            t0 = ts[0]
            i0 = MIDX[(m, t0)]
            nt = len(ts)
            kh = _dot(KC[:, t0 * 128:(t0 + nt) * 128].astype(bf), MM[i0 * 128:(i0 + nt) * 128, :])
            KH[m] = kh.astype(bf)

        cp_u.wait()

        def s3(j, c):
            cs = pl.ds(pl.multiple_of(j * 128, 128), 128)
            xn, rs = _ln0(U[:, cs].astype(f32))
            xb = xn.astype(bf)
            XNT[:, cs] = xb
            RS1[:, cs] = rs
            XH[j] = _dot(xb, Fm).astype(bf)
            return c
        _loop("s3", 16, s3)

        def s4(g, c):
            r = pl.ds(pl.multiple_of(g * 16, 16), 16)
            kv = [(KH[m, r, 0:128].astype(f32), KH[m, r, 128:256].astype(f32)) for m in range(16)]
            xv = [(XH[j, r, 0:128].astype(f32), XH[j, r, 128:256].astype(f32)) for j in range(16)]
            for i in range(16):
                yr = yi = None
                for j in range(i + 1):
                    tr, ti = _cmul(*kv[i - j], *xv[j])
                    yr = tr if yr is None else yr + tr
                    yi = ti if yi is None else yi + ti
                YH[i, r, 0:128] = yr.astype(bf)
                YH[i, r, 128:256] = yi.astype(bf)
            return c
        _loop("s4", 36, s4)

        def s6(i, c):
            cs = pl.ds(pl.multiple_of(i * 128, 128), 128)
            y = _dot(YH[i], Fm, NT)
            h = U[:, cs].astype(f32) + y + XNT[:, cs].astype(f32) * DSC[...]
            hn, rs = _ln0(h)
            hb = hn.astype(bf)
            HT[:, cs] = h.astype(bf)
            HNT[:, cs] = hb
            RS2[:, cs] = rs
            HN[cs, :] = hb.T
            return c
        _loop("s6", 16, s6)

    pl.run_scoped(ssm_fwd, pltpu.VMEM((D, 768), f32), pltpu.VMEM((16, D, 256), bf))

    cp_do.wait()
    cp_wout.wait()

    def tr_do(j, c):
        cs = pl.ds(pl.multiple_of(j * 256, 256), 256)
        DO[cs, :] = DOT_[:, cs].T
        return c
    _loop("tr_do", 8, tr_do)


    cp_win.wait()
    BS = 256

    def gmlp(T2, WT):
        def p2a(rb, c):
            rs_ = pl.ds(pl.multiple_of(rb * BS, BS), BS)
            hn = HN[rs_, :]
            do = DO[rs_, :]
            ssum = None
            for ft in range(9):
                fs = slice(ft * 256, (ft + 1) * 256)
                zp = _dot(hn, WIN[:, FH + ft * 256:FH + (ft + 1) * 256])
                z2, gd = _gelu_both(zp)
                T2[:, fs] = z2
                GD2[rs_, fs] = gd.astype(bf)
                part = z2[:, 0:128] + z2[:, 128:256]
                ssum = part if ssum is None else ssum + part
            mean = jnp.sum(ssum, axis=1, keepdims=True) * (1.0 / FH)
            sq = None
            for ft in range(18):
                fs = slice(ft * 128, (ft + 1) * 128)
                zc = T2[:, fs] - mean
                part = zc * zc
                sq = part if sq is None else sq + part
            r2 = lax.rsqrt(jnp.sum(sq, axis=1, keepdims=True) * (1.0 / FH) + EPS)
            RSG = None
            for ft in range(9):
                fs = slice(ft * 256, (ft + 1) * 256)
                Z2N[rs_, fs] = ((T2[:, fs] - mean) * r2).astype(bf)
            R2C[rs_, :] = jnp.broadcast_to(r2, (BS, 128))
            dsum = None
            for ft in range(9):
                fs = slice(ft * 256, (ft + 1) * 256)
                zp = _dot(hn, WIN[:, fs])
                z1, gd = _gelu_both(zp)
                z1b = z1.astype(bf)
                dp = _dot(do, WOUTT[:, fs])
                dg = (dp * z1b.astype(f32)).astype(bf)
                Z1[rs_, fs] = z1b
                DG[rs_, fs] = dg
                Q1[rs_, fs] = (dp * gd).astype(bf)
                dgf = dg.astype(f32)
                part = dgf[:, 0:128] + dgf[:, 128:256]
                dsum = part if dsum is None else dsum + part
            db = jnp.sum(dsum, axis=1, keepdims=True)
            DBROW[:, rs_] = jnp.broadcast_to(db, (BS, 128)).T[0:8, :]
            return c
        _loop("p2a", L // BS, p2a)

        cp_wsp.wait()

        def p2b(rb, c):
            rs_ = pl.ds(pl.multiple_of(rb * BS, BS), BS)
            wr = WSP[rs_, :]
            bc = BCOL[rs_, :]
            bc2 = jnp.concatenate([bc, bc], axis=1)
            for ft in range(9):
                fs = slice(ft * 256, (ft + 1) * 256)
                g = _dot(wr, Z2N[:, fs]) + bc2
                Z1[rs_, fs] = (Z1[rs_, fs].astype(f32) * g).astype(bf)
                Q1[rs_, fs] = (Q1[rs_, fs].astype(f32) * g).astype(bf)
            WT[...] = WSP[:, rs_].T
            wt = WT[...]
            s1 = s2 = None
            for ft in range(9):
                fs = slice(ft * 256, (ft + 1) * 256)
                dz = _dot(wt, DG[:, fs])
                T2[:, fs] = dz
                pz = dz * Z2N[rs_, fs].astype(f32)
                a = dz[:, 0:128] + dz[:, 128:256]
                b = pz[:, 0:128] + pz[:, 128:256]
                s1 = a if s1 is None else s1 + a
                s2 = b if s2 is None else s2 + b
            c1 = jnp.sum(s1, axis=1, keepdims=True) * (1.0 / FH)
            c2 = jnp.sum(s2, axis=1, keepdims=True) * (1.0 / FH)
            r2 = R2C[rs_, :][:, 0:1]
            for ft in range(9):
                fs = slice(ft * 256, (ft + 1) * 256)
                dz2 = r2 * (T2[:, fs] - c1 - Z2N[rs_, fs].astype(f32) * c2) * GD2[rs_, fs].astype(f32)
                GD2[rs_, fs] = dz2.astype(bf)
            outT = _dot(WOUTT[...], Z1[rs_, :], NT)
            h2 = HT[:, rs_].astype(f32) + outT
            U[:, rs_] = h2.astype(bf)
            pltpu.make_async_copy(U.at[:, rs_], h2_hbm.at[:, rs_], sem_out.at[rb]).start()
            dhn = _dot(WIN[:, 0:FH], Q1[rs_, :], NT) + _dot(WIN[:, FH:2 * FH], GD2[rs_, :], NT)
            hn = HNT[:, rs_].astype(f32)
            a1 = jnp.sum(dhn, axis=0, keepdims=True) * (1.0 / D)
            a2 = jnp.sum(dhn * hn, axis=0, keepdims=True) * (1.0 / D)
            dh = RS2[:, rs_] * (dhn - a1 - hn * a2) + DOT_[:, rs_].astype(f32)
            DHT[:, rs_] = dh.astype(bf)
            return c
        _loop("p2b", L // BS, p2b)

    def gmlp_outer(T2, WT, R2C_):
        nonlocal R2C
        R2C = R2C_
        gmlp(T2, WT)
    R2C = None
    pl.run_scoped(gmlp_outer, pltpu.VMEM((BS, FH), f32), pltpu.VMEM((BS, L), bf), pltpu.VMEM((L, 128), f32))

    def ssm_bwd(DY, DXH, DKH, DKC, DDT):
        def f1(j, c):
            cs = pl.ds(pl.multiple_of(j * 128, 128), 128)
            DY[j] = _dot(DHT[:, cs], Fm).astype(bf)
            return c
        _loop("f1", 16, f1)

        def f2(g, c):
            r = pl.ds(pl.multiple_of(g * 16, 16), 16)
            ld = lambda R, m: (R[m, r, 0:128].astype(f32), R[m, r, 128:256].astype(f32))
            kv = [ld(KH, m) for m in range(16)]
            xv = [ld(XH, m) for m in range(16)]
            dv = [ld(DY, m) for m in range(16)]
            for j in range(16):
                xr = xi = None
                for i in range(j, 16):
                    kr, ki = kv[i - j]
                    yr, yi = dv[i]
                    tr = kr * yr + ki * yi
                    ti = kr * yi - ki * yr
                    xr = tr if xr is None else xr + tr
                    xi = ti if xi is None else xi + ti
                DXH[j, r, 0:128] = xr.astype(bf)
                DXH[j, r, 128:256] = xi.astype(bf)
            for m in range(16):
                kr_ = ki_ = None
                for j in range(16 - m):
                    xr, xi = xv[j]
                    yr, yi = dv[j + m]
                    tr = xr * yr + xi * yi
                    ti = xr * yi - xi * yr
                    kr_ = tr if kr_ is None else kr_ + tr
                    ki_ = ti if ki_ is None else ki_ + ti
                DKH[m, r, 0:128] = kr_.astype(bf)
                DKH[m, r, 128:256] = ki_.astype(bf)
            return c
        _loop("f2", 36, f2)

        def f3(j, c):
            cs = pl.ds(pl.multiple_of(j * 128, 128), 128)
            dh = DHT[:, cs].astype(f32)
            xn = XNT[:, cs].astype(f32)
            dxn = _dot(DXH[j], Fm, NT) + dh * DSC[...]
            b1 = jnp.sum(dxn, axis=0, keepdims=True) * (1.0 / D)
            b2 = jnp.sum(dxn * xn, axis=0, keepdims=True) * (1.0 / D)
            du = dh + RS1[:, cs] * (dxn - b1 - xn * b2)
            DUT[:, cs] = du.astype(bf)
            return c + dh * xn
        with jax.named_scope("f3"):
            dsk_acc = lax.fori_loop(0, 16, f3, jnp.zeros((D, 128), f32))
        cp_du = pltpu.make_async_copy(DUT, du_hbm, sem_out.at[8])
        cp_du.start()
        dsk = jnp.sum(dsk_acc, axis=1, keepdims=True)
        dD_ref[...] = jnp.broadcast_to(dsk, (D, 128)).T[0, :].astype(bf)

        for t in range(6):
            ms = [m for (m, tt) in MKEYS if tt == t]
            acc = None
            for m in ms:
                i0 = MIDX[(m, t)]
                part = _dot(DKH[m], MM[i0 * 128:(i0 + 1) * 128, :], NT)
                acc = part if acc is None else acc + part
            DKC[:, t * 128:(t + 1) * 128] = acc

        def f4_group(g):
            r = pl.ds(pl.multiple_of(g * 8, 8), 8)
            l8 = (PAR[10, r, :], PAR[11, r, :])
            E = [(jnp.ones((8, 128), f32), jnp.zeros((8, 128), f32)), l8]
            for b in range(2, 16):
                E.append(_cmul(*E[-1], *l8))
            rhs = jnp.concatenate(
                [jnp.concatenate([e[0] for e in E], axis=0).astype(bf),
                 jnp.concatenate([e[1] for e in E], axis=0).astype(bf)], axis=1)
            rows = []
            for i in range(NB):
                t, slot = divmod(i, 8)
                x = DKC[r, t * 128:(t + 1) * 128]
                rr = pltpu.roll(x, 120 - slot, 1, stride=1, stride_axis=0)
                cpl = jnp.where(diag_mask, rr, 0.0)
                rows.append(cpl)
                rows.append(cpl * (lane8 + float(BASES[i])))
            lhs = jnp.concatenate(rows, axis=0).astype(bf)
            out = _dot(lhs, rhs)
            lam = {1: (PAR[2, r, :], PAR[3, r, :]), 2: (PAR[4, r, :], PAR[5, r, :]),
                   4: (PAR[6, r, :], PAR[7, r, :])}
            l128 = (PAR[8, r, :], PAR[9, r, :])
            res = []
            for w in range(2):
                def G(i):
                    return (out[16 * i + 8 * w:16 * i + 8 * w + 8, 0:128],
                            out[16 * i + 8 * w:16 * i + 8 * w + 8, 128:256])
                S = None
                idx = NB
                for m in range(16, -1, -1):
                    nb = 1 if m == 16 else 8 // _steps(m)
                    idx -= nb
                    inner = G(idx + nb - 1)
                    for a in range(nb - 2, -1, -1):
                        pr, pi = _cmul(*inner, *lam[_steps(m)])
                        gr, gi = G(idx + a)
                        inner = (pr + gr, pi + gi)
                    if S is None:
                        S = inner
                    else:
                        pr, pi = _cmul(*S, *l128)
                        S = (pr + inner[0], pi + inner[1])
                res.append(S)
            (s1r, s1i), (s2r, s2i) = res
            gWr, gWi = s1r, -s1i
            dt = DTC[r, :]
            wr, wi = PAR[0, r, :], PAR[1, r, :]
            gar = wr * s2r - wi * s2i
            gai = -(wr * s2i + wi * s2r)
            Arv, Aiv = Ar_f(r)
            Brv, Biv, Crv, Civ = BC_f(r)
            OUTS[0, r, :] = dt * gar
            OUTS[1, r, :] = dt * gai
            OUTS[2, r, :] = dt * (gWr * Crv + gWi * Civ)
            OUTS[3, r, :] = dt * (gWi * Crv - gWr * Civ)
            OUTS[4, r, :] = dt * (gWr * Brv + gWi * Biv)
            OUTS[5, r, :] = dt * (gWi * Brv - gWr * Biv)
            tot = dt * (gar * Arv + gai * Aiv) + (gWr * wr + gWi * wi)
            DDT[r, :] = jnp.broadcast_to(jnp.sum(tot, axis=1, keepdims=True), (8, 128))

        def cvt(i, c):
            r = pl.ds(pl.multiple_of(i * 64, 64), 64)
            for k, R in enumerate((Ar_ref, Ai_ref, Br_ref, Bi_ref, Cr_ref, Ci_ref)):
                PF[k, r, :] = R[r, :].astype(f32)
            return c
        _loop("cvt", 9, cvt)
        Ar_f = lambda r: (PF[0, r, :], PF[1, r, :])
        BC_f = lambda r: (PF[2, r, :], PF[3, r, :], PF[4, r, :], PF[5, r, :])

        def f4(i, c):
            f4_group(2 * i)
            f4_group(2 * i + 1)
            return c
        _loop("f4", 36, f4)
        for k, R in enumerate((dAr_ref, dAi_ref, dBr_ref, dBi_ref, dCr_ref, dCi_ref)):
            R[...] = OUTS[k].astype(bf)
        dlog_ref[...] = DDT[...].T[0, :].astype(bf)
        dbsp_ref[...] = DBROW[0, :].astype(bf)

    def ssm_bwd_outer(DY, DXH, DKH, DKC, DDT, PF_, OUTS_):
        nonlocal PF, OUTS
        PF, OUTS = PF_, OUTS_
        ssm_bwd(DY, DXH, DKH, DKC, DDT)
    PF = OUTS = None
    pl.run_scoped(ssm_bwd_outer, pltpu.VMEM((16, D, 256), bf), pltpu.VMEM((16, D, 256), bf),
                  pltpu.VMEM((16, D, 256), bf), pltpu.VMEM((D, 768), f32), pltpu.VMEM((D, 128), f32),
                  pltpu.VMEM((6, D, 128), f32), pltpu.VMEM((6, D, 128), f32))

    def g_wsp(rb, c):
        rs_ = pl.ds(pl.multiple_of(rb * BS, BS), BS)
        WSP[rs_, :] = _dot(DG[rs_, :], Z2N[...], NT).astype(bf)
        pltpu.make_async_copy(WSP.at[rs_, :], dwsp_hbm.at[rs_, :], sem_out.at[9 + rb]).start()
        return c
    _loop("g_wsp", L // BS, g_wsp)

    for half, R in enumerate((Q1, GD2)):
        def g_win(ct, c, half=half, R=R):
            cs = pl.ds(pl.multiple_of(ct * 256, 256), 256)
            co = pl.ds(pl.multiple_of(half * FH + ct * 256, 256), 256)
            WIN[:, co] = _dot(HNT[...], R[:, cs]).astype(bf)
            pltpu.make_async_copy(WIN.at[:, co], dwin_hbm.at[:, co], sem_out.at[17 + half * 9 + ct]).start()
            return c
        _loop("g_win%d" % half, 9, g_win)

    def g_wout(ct, c):
        cs = pl.ds(pl.multiple_of(ct * 256, 256), 256)
        WOUTT[:, cs] = _dot(DOT_[...], Z1[:, cs]).astype(bf)
        pltpu.make_async_copy(WOUTT.at[:, cs], dwout_hbm.at[:, cs], sem_out.at[35 + ct]).start()
        return c
    _loop("g_wout", 9, g_wout)

    for rb in range(8):
        rs_ = pl.ds(rb * BS, BS)
        pltpu.make_async_copy(U.at[:, rs_], h2_hbm.at[:, rs_], sem_out.at[rb]).wait()
        pltpu.make_async_copy(WSP.at[rs_, :], dwsp_hbm.at[rs_, :], sem_out.at[9 + rb]).wait()
    pltpu.make_async_copy(DUT, du_hbm, sem_out.at[8]).wait()
    for half in range(2):
        for ct in range(9):
            co = pl.ds(half * FH + ct * 256, 256)
            pltpu.make_async_copy(WIN.at[:, co], dwin_hbm.at[:, co], sem_out.at[17 + half * 9 + ct]).wait()
    for ct in range(9):
        cs = pl.ds(ct * 256, 256)
        pltpu.make_async_copy(WOUTT.at[:, cs], dwout_hbm.at[:, cs], sem_out.at[35 + ct]).wait()


@jax.jit
def pallas_sequential_preLN__ssm_conv_s4__mixer_gmlp__prompt_kernel(A_u, A_A_re, A_A_im, A_B_re, A_B_im, A_C_re, A_C_im, A_log_dt, A_Dskip,
        B_x, B_w_in, B_w_sp, B_b_sp, B_w_out, grad_out):
    u2 = A_u.reshape(L, D).T
    do2 = grad_out.reshape(L, D).T
    mcat = jnp.asarray(MCAT_NP, dtype=bf)
    fm = jnp.asarray(F_NP, dtype=bf)
    anyspec = pl.BlockSpec(memory_space=pl.ANY)
    vspec = pl.BlockSpec(memory_space=pltpu.VMEM)
    sds = jax.ShapeDtypeStruct
    out_shape = [sds((D, L), bf), sds((D, L), bf)] + [sds((D, N), bf)] * 6 + [
        sds((D,), bf), sds((D,), bf), sds((D, 2 * FH), bf), sds((L, L), bf), sds((L,), bf), sds((D, FH), bf)]
    out_specs = [anyspec, anyspec] + [vspec] * 6 + [vspec, vspec, anyspec, anyspec, vspec, anyspec]
    V = pltpu.VMEM
    scratch = [
        V((D, L), bf), V((L, D), bf), V((D, 2 * FH), bf), V((L, L), bf), V((D, FH), bf),
        V((len(MKEYS) * 128, 256), bf),
        V((D, L), bf), V((D, L), bf), V((D, L), bf), V((L, D), bf), V((D, L), bf), V((D, L), bf),
        V((L, FH), bf), V((L, FH), bf), V((L, FH), bf), V((L, FH), bf), V((L, FH), bf),
        V((16, D, 256), bf), V((16, D, 256), bf),
        V((14, D, 128), f32), V((D, 128), f32), V((D, 128), f32), V((L, 128), f32),
        V((1, L), f32), V((1, L), f32), V((8, L), f32),
        pltpu.SemaphoreType.DMA((8,)), pltpu.SemaphoreType.DMA((48,)),
    ]
    outs = pl.pallas_call(
        kernel,
        out_shape=out_shape,
        in_specs=[anyspec] * 6 + [vspec] * 10,
        out_specs=out_specs,
        scratch_shapes=scratch,
        compiler_params=pltpu.CompilerParams(vmem_limit_bytes=128 * 2**20),
        name="s4_gmlp_fwd_bwd",
    )(u2, do2, B_w_in, B_w_sp, B_w_out.T, mcat,
      A_A_re, A_A_im, A_B_re, A_B_im, A_C_re, A_C_im,
      A_log_dt, A_Dskip, B_b_sp, fm)
    (h2, du, dAr, dAi, dBr, dBi, dCr, dCi, dlog, dD, dwin, dwsp, dbsp, dwout) = outs
    return (h2.T.reshape(1, L, D), du.T.reshape(1, L, D), dAr, dAi, dBr, dBi, dCr, dCi,
            dlog, dD, dwin, dwsp, dbsp, dwout.T)
```

```python
import functools
import numpy as np
import jax
import jax.numpy as jnp
from jax import lax
import jax.experimental.pallas as pl
import jax.experimental.pallas.tpu as pltpu

bf = jnp.bfloat16
f32 = jnp.float32
L = 2048
D = 576
N = 128
T = 128
NC = 16
FH = 2304
EPS = 1e-5
C0 = float(np.sqrt(2.0 / np.pi))
C1 = 0.044715 * C0

NN = (((1,), (0,)), ((), ()))
NT = (((1,), (1,)), ((), ()))
TN = (((0,), (0,)), ((), ()))


def _bf16_round_np(a):
    a = np.ascontiguousarray(np.asarray(a, dtype=np.float32))
    u = a.view(np.uint32).astype(np.uint64)
    r = ((u + 0x7FFF + ((u >> 16) & 1)) >> 16) << 16
    return r.astype(np.uint32).view(np.float32)


def _build_consts():
    lt = _bf16_round_np(np.arange(L)).astype(np.int64)
    bases = []
    for m in range(16):
        step = 1 if m < 2 else 2 if m < 4 else 4 if m < 8 else 8
        for a in range(0, 8, step):
            bases.append(128 * m + a)
    bases.append(2048)
    pos = {}
    valid = set(lt.tolist())
    for i, bs in enumerate(bases):
        t, slot = divmod(i, 8)
        for b in range(16):
            v = bs + 8 * b
            if v in valid:
                assert v not in pos
                pos[v] = (t, 8 * ((b + 1) % 16) + slot)
    assert set(pos.keys()) == valid
    theta = np.pi * (2 * np.arange(T) + 1) / (2 * T)
    tau = np.arange(T)
    Fm = np.concatenate([np.cos(np.outer(tau, theta)), -np.sin(np.outer(tau, theta))], 1)
    Mp = {}
    for m in range(16):
        for l in range(max(0, 128 * m - 127), min(L, 128 * m + 128)):
            r = l - 128 * m
            t, ln = pos[int(lt[l])]
            M = Mp.setdefault((m, t), np.zeros((128, 256)))
            M[ln, :128] += np.cos(theta * r) / T
            M[ln, 128:] += -np.sin(theta * r) / T
    keys = sorted(Mp.keys())
    Mcat = np.concatenate([Mp[k] for k in keys], 0)
    return bases, keys, Mcat.astype(np.float32), Fm.astype(np.float32)


BASES, MKEYS, MCAT_NP, F_NP = _build_consts()
NB = len(BASES)
MIDX = {k: i for i, k in enumerate(MKEYS)}


def _dot(a, b, dims=NN):
    return lax.dot_general(a, b, dims, preferred_element_type=f32)


def _cmul(ar, ai, br, bi):
    return ar * br - ai * bi, ar * bi + ai * br


def _csq(ar, ai):
    return ar * ar - ai * ai, 2.0 * ar * ai


def _gelu_both(x):
    x2 = x * x
    u = x * (C0 + C1 * x2)
    th = jnp.tanh(u)
    hx = 0.5 * x
    s = 1.0 + th
    return hx * s, 0.5 * s + hx * (1.0 - th * th) * (C0 + (3.0 * C1) * x2)


def _gelu(x):
    x2 = x * x
    hx = 0.5 * x
    return hx + hx * jnp.tanh(x * (C0 + C1 * x2))


def _ln0(x):
    m = jnp.sum(x, axis=0, keepdims=True) * (1.0 / D)
    xc = x - m
    v = jnp.sum(xc * xc, axis=0, keepdims=True) * (1.0 / D)
    r = lax.rsqrt(v + EPS)
    return xc * r, r


def _loop(name, n, body, unroll=1):
    assert n % unroll == 0

    def outer(i, c):
        for q in range(unroll):
            body(i * unroll + q, c)
        return c
    with jax.named_scope(name):
        lax.fori_loop(0, n // unroll, outer, 0)


def _steps(m):
    return 1 if m < 2 else 2 if m < 4 else 4 if m < 8 else 8


TICK_P = 1000003
UNR = {"f2": 1, "s4": 2, "s1b": 6, "f3": 4, "s3": 2, "s1a": 2}


def _tick(t):
    return lax.rem(t, jnp.int32(TICK_P))


def kernel(u_hbm, do_hbm, win_hbm, wsp_hbm, wout_hbm, m_hbm,
           Ar_ref, Ai_ref, Br_ref, Bi_ref, Cr_ref, Ci_ref, logdt_ref, dsk_ref, bsp_ref, F_ref,
           h2_hbm, du_hbm, dAr_hbm, dAi_hbm, dBr_hbm, dBi_hbm, dCr_hbm, dCi_hbm, dlog_ref, dD_ref,
           dwin_hbm, dwsp_hbm, dbsp_ref, dwout_hbm,
           U, YH, WIN, WSP, WOUTT, MM, XNT, HT, HNT, DOT_, DHT,
           DZ, XH, KH, PAR, DTC, DSC, BCOL, RS1, RS2, DBROW, R2ROW, MRROW,
           sem_in, sem_h2, sem_du, sem_wsp, sem_win, sem_wout, sem_par):
    BS = 256
    DUT = HT
    DY = YH
    Q1 = DZ.at[:, 0:FH]
    GD2 = DZ.at[:, FH:2 * FH]

    def cin(src, dst, i):
        return pltpu.make_async_copy(src, dst, sem_in.at[i])

    cp_u = cin(u_hbm, U, 0)
    cp_do = cin(do_hbm, DOT_, 1)
    cp_wo8 = cin(wout_hbm.at[:, 8 * 256:FH], WOUTT.at[:, 8 * 256:FH], 2)
    cp_wout = cin(wout_hbm.at[:, 0:8 * 256], WOUTT.at[:, 0:8 * 256], 3)
    cp_m = cin(m_hbm, MM, 4)
    cp_win = cin(win_hbm, WIN, 5)
    cp_wsp = cin(wsp_hbm, WSP, 6)
    for c in (cp_u, cp_do, cp_wo8, cp_wout, cp_m, cp_win, cp_wsp):
        c.start()

    Fm = F_ref[...]

    dt_row = jnp.exp(logdt_ref[...].astype(f32)[None, :]).astype(bf).astype(f32)
    DTC[...] = jnp.broadcast_to(dt_row, (128, D)).T
    DSC[...] = jnp.broadcast_to(dsk_ref[...].astype(f32)[None, :], (128, D)).T
    bsp_row = bsp_ref[...].astype(f32)[None, :]
    for i in range(16):
        BCOL[i * 128:(i + 1) * 128, :] = jnp.broadcast_to(bsp_row[:, i * 128:(i + 1) * 128], (128, 128)).T

    def s0(i, c):
        r = pl.ds(pl.multiple_of(i * 64, 64), 64)
        dt = DTC[r, :]
        ar = dt * Ar_ref[r, :].astype(f32)
        ai = dt * Ai_ref[r, :].astype(f32)
        cbr, cbi = _cmul(Cr_ref[r, :].astype(f32), Ci_ref[r, :].astype(f32),
                         Br_ref[r, :].astype(f32), Bi_ref[r, :].astype(f32))
        PAR[0, r, :] = dt * cbr
        PAR[1, r, :] = dt * cbi
        e = jnp.exp(ar)
        l1 = (e * jnp.cos(ai), e * jnp.sin(ai))
        l2 = _csq(*l1)
        l4 = _csq(*l2)
        l8 = _csq(*l4)
        l128 = _csq(*_csq(*_csq(*_csq(*l8))))
        for k, z in enumerate((l1, l2, l4, l128, l8)):
            PAR[2 + 2 * k, r, :] = z[0]
            PAR[3 + 2 * k, r, :] = z[1]
        return c
    _loop("s0", 9, s0)
    for c in range(8):
        PAR[12, pl.ds(c, 72, stride=8), :] = PAR[10, pl.ds(7 - c, 72, stride=8), :]
        PAR[13, pl.ds(c, 72, stride=8), :] = -PAR[11, pl.ds(7 - c, 72, stride=8), :]

    lane = lax.broadcasted_iota(jnp.int32, (8, 128), 1)
    subl = lax.broadcasted_iota(jnp.int32, (8, 128), 0)
    slot_mask = [(lane & 7) == s for s in range(8)]
    diag_mask = (lane & 7) == subl
    lane8 = ((lane >> 3) * 8).astype(f32)

    def powers16(l8):
        E = [(jnp.ones((8, 128), f32), jnp.zeros((8, 128), f32)), l8]
        for b in range(2, 16):
            E.append(_cmul(*E[-1], *l8))
        return jnp.concatenate(
            [jnp.concatenate([e[0] for e in E], axis=0).astype(bf),
             jnp.concatenate([e[1] for e in E], axis=0).astype(bf)], axis=1)

    def step_ratios(r):
        return {1: (PAR[2, r, :], PAR[3, r, :]), 2: (PAR[4, r, :], PAR[5, r, :]), 4: (PAR[6, r, :], PAR[7, r, :])}

    def gated_lhs(ref, ts, base, ktiles):
        nk = ref.shape[1] // 128
        rows = ref.shape[0]
        gate = dict(zip(ktiles, ts))
        cols = []
        k0 = 0
        for k in sorted(gate) + [nk]:
            if k > k0:
                cols.append(ref[:, k0 * 128:k * 128])
            if k < nk:
                half = rows // 2
                cols.append(jnp.concatenate(
                    [ref[pl.ds(pl.multiple_of((gate[k] - base) * 16 + q * half, 16), half), k * 128:(k + 1) * 128]
                     for q in range(2)], axis=0))
            k0 = k + 1
        return jnp.concatenate(cols, axis=1)

    def ticks(t, n):
        out = []
        for _ in range(n):
            t = _tick(t)
            out.append(t)
        return out

    def rows16(t):
        return pl.ds(pl.multiple_of(t * 16, 16), 16)

    def ssm_fwd(KC, DO, KH32, XH32):
        def dp_cols(rb, col0, ncol):
            rs_ = pl.ds(pl.multiple_of(rb * BS, BS), BS)
            cn = pl.ds(pl.multiple_of(col0, 128), ncol)
            DZ[rs_, cn] = _dot(DO[rs_, :], WOUTT[:, cn]).astype(bf)

        def s1_group(g):
            r = pl.ds(pl.multiple_of(g * 8, 8), 8)
            rhs = powers16((PAR[12, r, :], PAR[13, r, :]))
            lam = step_ratios(r)
            l128 = (PAR[8, r, :], PAR[9, r, :])
            cur = (PAR[0, r, :], PAR[1, r, :])
            Us = []
            for m in range(17):
                z = cur
                if m < 16:
                    st = _steps(m)
                    for a in range(0, 8, st):
                        Us.append(z)
                        if a + st < 8:
                            z = _cmul(*z, *lam[st])
                    cur = _cmul(*cur, *l128)
                else:
                    Us.append(z)
            zero = jnp.zeros((8, 128), f32)
            lhs = jnp.concatenate(
                [jnp.concatenate([x[0] for x in Us] + [zero], axis=0).astype(bf),
                 jnp.concatenate([x[1] for x in Us] + [zero], axis=0).astype(bf)], axis=1)
            out = _dot(lhs, rhs, NT)
            for t in range(6):
                acc = None
                for slot in range(8):
                    i = 8 * t + slot
                    if i >= NB:
                        break
                    rr = pltpu.roll(out[8 * i:8 * i + 8, :], slot + 1, 1, stride=1, stride_axis=0)
                    acc = jnp.where(slot_mask[slot], rr, 0.0 if acc is None else acc)
                KC[r, t * 128:(t + 1) * 128] = acc

        NS1A = 8

        def s1a(i, c):
            for q in range(4):
                s1_group(4 * i + q)
            return c

        _loop("s1a", NS1A, s1a, 4)
        cp_u.wait()
        cp_do.wait()
        cp_wo8.wait()

        def s3(rb, c):
            rs_ = pl.ds(pl.multiple_of(rb * BS, BS), BS)
            dot_ = DOT_[:, rs_].T
            DO[rs_, :] = dot_
            DZ[rs_, 8 * 256:FH] = _dot(dot_, WOUTT[:, 8 * 256:FH]).astype(bf)
            for q in range(2):
                cs = pl.ds(pl.multiple_of(rb * BS + q * 128, 128), 128)
                xn, rs = _ln0(U[:, cs].astype(f32))
                XNT[:, cs] = xn.astype(bf)
                RS1[:, cs] = rs
            return c
        _loop("s3", 8, s3, UNR.get("s3", 1))
        cp_wout.wait()

        def s1b(i, c):
            g0 = 4 * (i + NS1A)
            t0 = 2 * i
            dp_cols(t0 // 16, (t0 % 16) * 128, 128)
            s1_group(g0)
            s1_group(g0 + 1)
            s1_group(g0 + 2)
            s1_group(g0 + 3)
            dp_cols(t0 // 16, (t0 % 16) * 128 + 128, 128)
            return c
        NB1 = 18 - NS1A
        _loop("s1b", NB1, s1b, 5)

        cp_m.wait()
        with jax.named_scope("s2"):
            for m in range(16):
                ts = [t for (mm, t) in MKEYS if mm == m]
                t0 = ts[0]
                i0 = MIDX[(m, t0)]
                nt = len(ts)
                kh = _dot(KC[:, t0 * 128:(t0 + nt) * 128].astype(bf), MM[i0 * 128:(i0 + nt) * 128, :])
                KH32[m] = kh
                KH[m] = kh.astype(bf)
            for j in range(16):
                xh = _dot(XNT[:, j * 128:(j + 1) * 128], Fm)
                XH32[j] = xh
                XH[j] = xh.astype(bf)

        NG4 = 6
        NT4 = 3 * NG4

        def s4(i, c):
            RC = 4
            pts = [(n, cc) for n in range(NT4) for cc in range(RC)][2:-2]
            t0 = NG4 * i
            ts = {}
            t = t0
            for p_ in pts:
                t = _tick(t)
                ts[p_] = t
            blocks = [(q, i0) for q in range(NG4) for i0 in range(14, -1, -2)]
            nsteps = sum(i0 + 2 for _, i0 in blocks)
            cnt = [0]

            def next_t():
                idx = cnt[0] * len(pts) // nsteps
                cnt[0] += 1
                return ts[pts[idx]]

            for q, i0 in blocks:
                acc = {}
                kc = {}
                r = None
                for j in range(i0 + 2):
                    r = rows16(next_t() + q)
                    x = (XH32[j, r, 0:128], XH32[j, r, 128:256])
                    xs = x[0] + x[1]
                    for ii in range(max(i0, j), i0 + 2):
                        m = ii - j
                        if m not in kc:
                            kr, ki = KH32[m, r, 0:128], KH32[m, r, 128:256]
                            kc[m] = (kr, ki, kr + ki)
                        t3 = (kc[m][0] * x[0], kc[m][1] * x[1], kc[m][2] * xs)
                        acc[ii] = tuple(a + b for a, b in zip(acc[ii], t3)) if ii in acc else t3
                for ii in range(i0, i0 + 2):
                    YH[ii, r, 0:128] = (acc[ii][0] - acc[ii][1]).astype(bf)
                    YH[ii, r, 128:256] = (acc[ii][2] - acc[ii][0] - acc[ii][1]).astype(bf)
            rcz = BS // RC
            for n in range(NT4):
                tile = 2 * NB1 + NT4 * i + n
                rb = tile // 16
                rs_ = pl.ds(pl.multiple_of(rb * BS, BS), BS)
                cn = pl.ds(pl.multiple_of((tile % 16) * 128, 128), 128)
                parts = []
                for cc in range(RC):
                    base = rb * BS + cc * rcz
                    if (n, cc) in ts:
                        base = base + (ts[(n, cc)] - t0)
                    parts.append(DO[pl.ds(pl.multiple_of(base, 16), rcz), 0:128])
                lhs = jnp.concatenate([jnp.concatenate(parts, axis=0), DO[rs_, 128:D]], axis=1)
                DZ[rs_, cn] = _dot(lhs, WOUTT[:, cn]).astype(bf)
            return c
        _loop("s4", 36 // NG4, s4)

    pl.run_scoped(ssm_fwd, pltpu.VMEM((D, 768), f32), pltpu.VMEM((L, D), bf),
                  pltpu.VMEM((16, D, 256), f32), pltpu.VMEM((16, D, 256), f32))

    def gmlp_and_bwd(Z1, Z2, DG, DBC):
        def gmlp(T2, WT, R2C, MRC, HN, ACC, DHN):
            def s6(i):
                cs = pl.ds(pl.multiple_of(i * 128, 128), 128)
                y = _dot(YH[i], Fm, NT)
                h = U[:, cs].astype(f32) + y + XNT[:, cs].astype(f32) * DSC[...]
                hn, rs = _ln0(h)
                hb = hn.astype(bf)
                HT[:, cs] = h.astype(bf)
                HNT[:, cs] = hb
                RS2[:, cs] = rs
                HN[cs, :] = hb.T

            with jax.named_scope("s6pro"):
                s6(0)
                s6(1)
            cp_win.wait()

            def p2a(rb, c, with_s6=True):
                rs_ = pl.ds(pl.multiple_of(rb * BS, BS), BS)
                hn = HN[rs_, :]
                for ft in range(9):
                    fs = slice(ft * 256, (ft + 1) * 256)
                    zp = _dot(hn, WIN[:, fs])
                    dgf = Q1[rs_, fs].astype(f32) * _gelu(zp)
                    Z1[rs_, fs] = zp.astype(bf)
                    DG[rs_, fs] = dgf.astype(bf)
                    part = dgf[:, 0:128] + dgf[:, 128:256]
                    if ft == 0:
                        ACC[0] = part
                    else:
                        ACC[0] += part
                db = jnp.sum(ACC[0], axis=1, keepdims=True)
                dbb = jnp.broadcast_to(db, (BS, 128))
                DBC[rs_, :] = dbb
                DBROW[:, rs_] = dbb.T[0:8, :]
                if with_s6:
                    s6(2 * rb + 2)
                for ft in range(9):
                    fs = slice(ft * 256, (ft + 1) * 256)
                    zp = _dot(hn, WIN[:, FH + ft * 256:FH + (ft + 1) * 256])
                    z2 = _gelu(zp)
                    Z2[rs_, fs] = z2.astype(bf)
                    GD2[rs_, fs] = zp.astype(bf)
                    zz = z2 * z2
                    p1 = z2[:, 0:128] + z2[:, 128:256]
                    p2 = zz[:, 0:128] + zz[:, 128:256]
                    if ft == 0:
                        ACC[1] = p1
                        ACC[2] = p2
                    else:
                        ACC[1] += p1
                        ACC[2] += p2
                    if ft == 3 and with_s6:
                        s6(2 * rb + 3)
                mean = jnp.sum(ACC[1], axis=1, keepdims=True) * (1.0 / FH)
                var = jnp.maximum(jnp.sum(ACC[2], axis=1, keepdims=True) * (1.0 / FH) - mean * mean, 0.0)
                r2 = lax.rsqrt(var + EPS)
                r2b = jnp.broadcast_to(r2, (BS, 128))
                mrb = jnp.broadcast_to(mean * r2, (BS, 128))
                R2C[rs_, :] = r2b
                MRC[rs_, :] = mrb
                R2ROW[:, rs_] = r2b.T[0:8, :]
                MRROW[:, rs_] = mrb.T[0:8, :]
                return c
            _loop("p2a", L // BS - 1, p2a)
            with jax.named_scope("p2a_last"):
                p2a(L // BS - 1, 0, with_s6=False)

            cp_wsp.wait()

            def prep_g(rb, offs=(0, 0)):
                n = BS // len(offs)
                for q, off in enumerate(offs):
                    rq = pl.ds(pl.multiple_of(rb * BS + q * n + off * 16, 16), n)
                    wf = WSP[rq, :].astype(f32)
                    WT[q * n:(q + 1) * n, :] = (wf * R2ROW[0:1, :]).astype(bf)
                    ACC[0, q * n:(q + 1) * n, :] = BCOL[rq, :] - jnp.sum(wf * MRROW[0:1, :], axis=1, keepdims=True)

            prep_g(0)

            def p2b(rb, c):
                rs_ = pl.ds(pl.multiple_of(rb * BS, BS), BS)
                wr = WT[...]
                bc = ACC[0][:, 0:1]
                for ft in range(9):
                    fs = slice(ft * 256, (ft + 1) * 256)
                    g = _dot(wr, Z2[:, fs]) + bc
                    z1, gd1 = _gelu_both(Z1[rs_, fs].astype(f32))
                    Z1[rs_, fs] = (z1 * g).astype(bf)
                    Q1[rs_, fs] = (Q1[rs_, fs].astype(f32) * gd1 * g).astype(bf)
                ts = ticks(rb, 4)
                prep_g(jnp.minimum(rb + 1, L // BS - 1), [t - rb for t in ts])
                outT = _dot(gated_lhs(WOUTT, ts, rb, (1, 4, 7, 10)), Z1[rs_, :], NT)
                h2 = HT[:, rs_].astype(f32) + outT
                U[:, rs_] = h2.astype(bf)
                pltpu.make_async_copy(U.at[:, rs_], h2_hbm.at[:, rs_], sem_h2.at[rb]).start()
                return c
            _loop("p2b", L // BS, p2b)

            def prep_t(rb, offs=(0,)):
                n = L // len(offs)
                for q, off in enumerate(offs):
                    WT[:, q * n:(q + 1) * n] = WSP[q * n:(q + 1) * n,
                                                   pl.ds(pl.multiple_of(rb * BS + off * 128, 128), BS)].T

            def fin_dh(rb):
                rs_ = pl.ds(pl.multiple_of(rb * BS, BS), BS)
                dhn = DHN[...]
                hn = HNT[:, rs_].astype(f32)
                a1 = jnp.sum(dhn, axis=0, keepdims=True) * (1.0 / D)
                a2 = jnp.sum(dhn * hn, axis=0, keepdims=True) * (1.0 / D)
                dh = RS2[:, rs_] * (dhn - a1 - hn * a2) + DOT_[:, rs_].astype(f32)
                DHT[:, rs_] = dh.astype(bf)

            def dy_hat(rb):
                for q in range(2):
                    cs = pl.ds(pl.multiple_of(rb * BS + q * 128, 128), 128)
                    DY[2 * rb + q] = _dot(DHT[:, cs], Fm).astype(bf)

            prep_t(0)
            DHN[...] = jnp.zeros((D, BS), f32)
            DHT[:, 0:BS] = jnp.zeros((D, BS), bf)

            def p2c(rb, c):
                rs_ = pl.ds(pl.multiple_of(rb * BS, BS), BS)
                dprev = [DHT[:, pl.ds(pl.multiple_of(jnp.maximum(rb - 2, 0) * BS + q * 128, 128), 128)]
                         for q in range(2)]
                fin_dh(jnp.maximum(rb - 1, 0))
                wt = WT[...]
                s1 = s2 = None
                for ft in range(9):
                    fs = slice(ft * 256, (ft + 1) * 256)
                    dz = _dot(wt, DG[:, fs])
                    T2[:, fs] = dz
                    pz = dz * Z2[rs_, fs].astype(f32)
                    a = dz[:, 0:128] + dz[:, 128:256]
                    b = pz[:, 0:128] + pz[:, 128:256]
                    s1 = a if s1 is None else s1 + a
                    s2 = b if s2 is None else s2 + b
                r2 = R2C[rs_, :][:, 0:1]
                mr = MRC[rs_, :][:, 0:1]
                c1 = jnp.sum(s1, axis=1, keepdims=True) * (1.0 / FH)
                c2 = jnp.sum(s2, axis=1, keepdims=True) * (1.0 / FH) * r2 - c1 * mr
                for ft in range(9):
                    fs = slice(ft * 256, (ft + 1) * 256)
                    z2n = Z2[rs_, fs].astype(f32) * r2 - mr
                    _, gd2 = _gelu_both(GD2[rs_, fs].astype(f32))
                    dz2 = r2 * (T2[:, fs] - c1 - z2n * c2) * gd2
                    GD2[rs_, fs] = dz2.astype(bf)
                ts = ticks(rb, 4)
                prep_t(jnp.minimum(rb + 1, L // BS - 1), [t - rb for t in ts])
                DHN[...] = _dot(gated_lhs(WIN, ts, rb, (20, 23, 26, 29)), DZ[rs_, :], NT)
                for q in range(2):
                    DY[2 * jnp.maximum(rb - 2, 0) + q] = _dot(dprev[q], Fm).astype(bf)
                return c
            _loop("p2c", L // BS, p2c)
            fin_dh(L // BS - 1)
            dy_hat(L // BS - 2)
            dy_hat(L // BS - 1)

        pl.run_scoped(gmlp, pltpu.VMEM((BS, FH), f32), pltpu.VMEM((BS, L), bf), pltpu.VMEM((L, 128), f32),
                      pltpu.VMEM((L, 128), f32), pltpu.VMEM((L, D), bf), pltpu.VMEM((3, BS, 128), f32),
                      pltpu.VMEM((D, BS), f32))

        def ssm_bwd(DXH, DKH, DKC, DDT, DDS, PF, OUTS):
            def ldc(R, m, r):
                return R[m, r, 0:128].astype(f32), R[m, r, 128:256].astype(f32)

            def lda(R, m, r):
                a = ldc(R, m, r)
                return a + (a[0] - a[1],)

            def ldb(R, m, r):
                b = ldc(R, m, r)
                return b + (b[0] + b[1],)

            def mac(acc, key, a, b):
                t = (a[0] * b[0], a[1] * b[1], a[2] * b[2])
                acc[key] = tuple(x + y for x, y in zip(acc[key], t)) if key in acc else t

            def cvt(i, c):
                r = pl.ds(pl.multiple_of(i * 64, 64), 64)
                for k, R in enumerate((Ar_ref, Ai_ref, Br_ref, Bi_ref, Cr_ref, Ci_ref)):
                    PF[k, r, :] = R[r, :].astype(f32)
                return c
            _loop("cvt", 9, cvt)

            NG2 = 4

            def f2(it, c):
                g0 = NG2 * it
                RC = 3
                pts = [(q, n, kq, cc) for q in range(NG2) for n in range(2) for kq in range(4)
                       for cc in range(RC)][1:-1]
                ts = {}
                t = g0
                for p_ in pts:
                    t = _tick(t)
                    ts[p_] = t
                blocks = []
                for q in range(NG2):
                    for i0 in range(0, 16, 2):
                        blocks += [(q, 0, i0), (q, 1, i0)]
                nsteps = sum(16 - i0 for _, _, i0 in blocks)
                cnt = [0]

                def next_t():
                    idx = cnt[0] * len(pts) // nsteps
                    cnt[0] += 1
                    return ts[pts[idx]]

                for q, kind, i0 in blocks:
                    acc = {}
                    cache = {}
                    r = None
                    if kind == 0:
                        for ii in range(i0, 16):
                            r = rows16(next_t() + q)
                            y = ldb(DY, ii, r)
                            for j in range(i0, min(ii, i0 + 1) + 1):
                                m = ii - j
                                if m not in cache:
                                    cache[m] = lda(KH, m, r)
                                mac(acc, j, cache[m], y)
                        dst = DXH
                    else:
                        for j in range(16 - i0):
                            r = rows16(next_t() + q)
                            x = lda(XH, j, r)
                            for m in range(i0, i0 + 2):
                                if j + m > 15:
                                    continue
                                if j + m not in cache:
                                    cache[j + m] = ldb(DY, j + m, r)
                                mac(acc, m, x, cache[j + m])
                        dst = DKH
                    for j in range(i0, i0 + 2):
                        dst[j, r, 0:128] = (acc[j][0] + acc[j][1]).astype(bf)
                        dst[j, r, 128:256] = (acc[j][2] - acc[j][0] + acc[j][1]).astype(bf)
                rcz = 288 // RC
                for q in range(NG2):
                    rh = q % 2
                    ct = (NG2 // 2) * it + q // 2
                    ro = slice(rh * 288, (rh + 1) * 288)
                    for n in range(2):
                        cn = pl.ds(pl.multiple_of(ct * 256 + n * 128, 128), 128)
                        cols = []
                        for kk in range(16):
                            parts = []
                            for cc in range(RC):
                                base = rh * 288 + cc * rcz
                                if kk % 4 == 0 and (q, n, kk // 4, cc) in ts:
                                    parts.append(HNT[pl.ds(pl.multiple_of(base + (ts[(q, n, kk // 4, cc)] - g0), 16),
                                                           rcz), kk * 128:(kk + 1) * 128])
                                else:
                                    parts.append(HNT[base:base + rcz, kk * 128:(kk + 1) * 128])
                            cols.append(jnp.concatenate(parts, axis=0))
                        WIN[ro, cn] = _dot(jnp.concatenate(cols, axis=1), DZ[:, cn]).astype(bf)
                    if rh == 1:
                        co = pl.ds(pl.multiple_of(ct * 256, 256), 256)
                        pltpu.make_async_copy(WIN.at[:, co], dwin_hbm.at[:, co], sem_win.at[ct]).start()
                return c
            _loop("f2", 36 // NG2, f2)

            with jax.named_scope("dkt"):
                for t in range(6):
                    ms = [m for (m, tt) in MKEYS if tt == t]
                    acc = None
                    for m in ms:
                        i0 = MIDX[(m, t)]
                        part = _dot(DKH[m], MM[i0 * 128:(i0 + 1) * 128, :], NT)
                        acc = part if acc is None else acc + part
                    DKC[:, t * 128:(t + 1) * 128] = acc

            def f4_group(g):
                r = pl.ds(pl.multiple_of(g * 8, 8), 8)
                rhs = powers16((PAR[10, r, :], PAR[11, r, :]))
                rows = []
                for i in range(NB):
                    t, slot = divmod(i, 8)
                    rr = pltpu.roll(DKC[r, t * 128:(t + 1) * 128], 120 - slot, 1, stride=1, stride_axis=0)
                    cpl = jnp.where(diag_mask, rr, 0.0)
                    rows.append(cpl)
                    rows.append(cpl * (lane8 + float(BASES[i])))
                lhs = jnp.concatenate(rows, axis=0).astype(bf)
                out = _dot(lhs, rhs)
                lam = step_ratios(r)
                l128 = (PAR[8, r, :], PAR[9, r, :])
                res = []
                for w in range(2):
                    def G(i):
                        return (out[16 * i + 8 * w:16 * i + 8 * w + 8, 0:128],
                                out[16 * i + 8 * w:16 * i + 8 * w + 8, 128:256])
                    S = None
                    idx = NB
                    for m in range(16, -1, -1):
                        nb = 1 if m == 16 else 8 // _steps(m)
                        idx -= nb
                        inner = G(idx + nb - 1)
                        for a in range(nb - 2, -1, -1):
                            pr, pi_ = _cmul(*inner, *lam[_steps(m)])
                            gr, gi = G(idx + a)
                            inner = (pr + gr, pi_ + gi)
                        if S is None:
                            S = inner
                        else:
                            pr, pi_ = _cmul(*S, *l128)
                            S = (pr + inner[0], pi_ + inner[1])
                    res.append(S)
                (s1r, s1i), (s2r, s2i) = res
                gWr, gWi = s1r, -s1i
                dt = DTC[r, :]
                wr, wi = PAR[0, r, :], PAR[1, r, :]
                gar = wr * s2r - wi * s2i
                gai = -(wr * s2i + wi * s2r)
                Arv, Aiv, Brv, Biv, Crv, Civ = [PF[k, r, :] for k in range(6)]
                OUTS[0, r, :] = dt * gar
                OUTS[1, r, :] = dt * gai
                OUTS[2, r, :] = dt * (gWr * Crv + gWi * Civ)
                OUTS[3, r, :] = dt * (gWi * Crv - gWr * Civ)
                OUTS[4, r, :] = dt * (gWr * Brv + gWi * Biv)
                OUTS[5, r, :] = dt * (gWi * Brv - gWr * Biv)
                tot = dt * (gar * Arv + gai * Aiv) + (gWr * wr + gWi * wi)
                DDT[r, :] = jnp.broadcast_to(jnp.sum(tot, axis=1, keepdims=True), (8, 128))

            def f4(rb, c):
                rs_ = pl.ds(pl.multiple_of(rb * BS, BS), BS)
                dgr = DG[rs_, :]
                dbc = DBC[rs_, :][:, 0:1]
                for k in range(9):
                    f4_group(9 * rb + k)
                    if k < 8:
                        ks = slice(k * 256, (k + 1) * 256)
                        a = _dot(dgr, Z2[ks, :], NT)
                        WSP[rs_, ks] = (a * R2ROW[0:1, ks] - dbc * MRROW[0:1, ks]).astype(bf)
                pltpu.make_async_copy(WSP.at[rs_, :], dwsp_hbm.at[rs_, :], sem_wsp.at[rb]).start()
                return c
            _loop("f4", 8, f4, 2)

            for k, R in enumerate((dAr_hbm, dAi_hbm, dBr_hbm, dBi_hbm, dCr_hbm, dCi_hbm)):
                KH[k, :, 0:128] = OUTS[k].astype(bf)
                pltpu.make_async_copy(KH.at[k, :, 0:128], R, sem_par.at[k]).start()
            dlog_ref[...] = DDT[...].T[0, :].astype(bf)
            dbsp_ref[...] = DBROW[0, :].astype(bf)

            def wout_tile(ct):
                cs = pl.ds(pl.multiple_of(ct * 256, 256), 256)
                WOUTT[:, cs] = _dot(DOT_[...], Z1[:, cs]).astype(bf)
                pltpu.make_async_copy(WOUTT.at[:, cs], dwout_hbm.at[:, cs], sem_wout.at[ct]).start()

            def f3(i, c):
                for q in range(2):
                    cs = pl.ds(pl.multiple_of((2 * i + q) * 128, 128), 128)
                    dh = DHT[:, cs].astype(f32)
                    xn = XNT[:, cs].astype(f32)
                    dxn = _dot(DXH[2 * i + q], Fm, NT) + dh * DSC[...]
                    b1 = jnp.sum(dxn, axis=0, keepdims=True) * (1.0 / D)
                    b2 = jnp.sum(dxn * xn, axis=0, keepdims=True) * (1.0 / D)
                    du = dh + RS1[:, cs] * (dxn - b1 - xn * b2)
                    DUT[:, cs] = du.astype(bf)
                    DDS[...] += dh * xn
                    WOUTT[:, cs] = _dot(DOT_[...], Z1[:, cs]).astype(bf)
                c2 = pl.ds(pl.multiple_of(i * 256, 256), 256)
                pltpu.make_async_copy(DUT.at[:, c2], du_hbm.at[:, c2], sem_du.at[i]).start()
                pltpu.make_async_copy(WOUTT.at[:, c2], dwout_hbm.at[:, c2], sem_wout.at[i]).start()
                return c
            DDS[...] = jnp.zeros((D, 128), f32)
            _loop("f3", 8, f3, UNR.get("f3", 1))
            dsk = jnp.sum(DDS[...], axis=1, keepdims=True)
            dD_ref[...] = jnp.broadcast_to(dsk, (D, 128)).T[0, :].astype(bf)
            wout_tile(8)

        pl.run_scoped(ssm_bwd, pltpu.VMEM((16, D, 256), bf), pltpu.VMEM((16, D, 256), bf),
                      pltpu.VMEM((D, 768), f32), pltpu.VMEM((D, 128), f32), pltpu.VMEM((D, 128), f32),
                      pltpu.VMEM((6, D, 128), f32), pltpu.VMEM((6, D, 128), f32))

    pl.run_scoped(gmlp_and_bwd, pltpu.VMEM((L, FH), bf), pltpu.VMEM((L, FH), bf), pltpu.VMEM((L, FH), bf),
                  pltpu.VMEM((L, 128), f32))

    for rb in range(8):
        rs_ = pl.ds(rb * BS, BS)
        pltpu.make_async_copy(U.at[:, rs_], h2_hbm.at[:, rs_], sem_h2.at[rb]).wait()
        pltpu.make_async_copy(WSP.at[rs_, :], dwsp_hbm.at[rs_, :], sem_wsp.at[rb]).wait()
        pltpu.make_async_copy(DUT.at[:, rs_], du_hbm.at[:, rs_], sem_du.at[rb]).wait()
    for ct in range(18):
        co = pl.ds(ct * 256, 256)
        pltpu.make_async_copy(WIN.at[:, co], dwin_hbm.at[:, co], sem_win.at[ct]).wait()
    for ct in range(9):
        cs = pl.ds(ct * 256, 256)
        pltpu.make_async_copy(WOUTT.at[:, cs], dwout_hbm.at[:, cs], sem_wout.at[ct]).wait()
    for k, R in enumerate((dAr_hbm, dAi_hbm, dBr_hbm, dBi_hbm, dCr_hbm, dCi_hbm)):
        pltpu.make_async_copy(KH.at[k, :, 0:128], R, sem_par.at[k]).wait()


@jax.jit
def pallas_sequential_preLN__ssm_conv_s4__mixer_gmlp__prompt_kernel(A_u, A_A_re, A_A_im, A_B_re, A_B_im, A_C_re, A_C_im, A_log_dt, A_Dskip,
        B_x, B_w_in, B_w_sp, B_b_sp, B_w_out, grad_out):
    u2 = A_u.reshape(L, D).T
    do2 = grad_out.reshape(L, D).T
    mcat = jnp.asarray(MCAT_NP, dtype=bf)
    fm = jnp.asarray(F_NP, dtype=bf)
    anyspec = pl.BlockSpec(memory_space=pl.ANY)
    vspec = pl.BlockSpec(memory_space=pltpu.VMEM)
    sds = jax.ShapeDtypeStruct
    out_shape = [sds((D, L), bf), sds((D, L), bf)] + [sds((D, N), bf)] * 6 + [
        sds((D,), bf), sds((D,), bf), sds((D, 2 * FH), bf), sds((L, L), bf), sds((L,), bf), sds((D, FH), bf)]
    out_specs = [anyspec] * 8 + [vspec, vspec, anyspec, anyspec, vspec, anyspec]
    V = pltpu.VMEM
    scratch = [
        V((D, L), bf), V((16, D, 256), bf), V((D, 2 * FH), bf), V((L, L), bf), V((D, FH), bf),
        V((len(MKEYS) * 128, 256), bf),
        V((D, L), bf), V((D, L), bf), V((D, L), bf), V((D, L), bf), V((D, L), bf),
        V((L, 2 * FH), bf), V((16, D, 256), bf), V((16, D, 256), bf),
        V((14, D, 128), f32), V((D, 128), f32), V((D, 128), f32), V((L, 128), f32),
        V((1, L), f32), V((1, L), f32), V((8, L), f32), V((8, L), f32), V((8, L), f32),
    ] + [pltpu.SemaphoreType.DMA((n,)) for n in (8, 8, 8, 8, 18, 9, 6)]
    outs = pl.pallas_call(
        kernel,
        out_shape=out_shape,
        in_specs=[anyspec] * 6 + [vspec] * 10,
        out_specs=out_specs,
        scratch_shapes=scratch,
        compiler_params=pltpu.CompilerParams(vmem_limit_bytes=128 * 2**20),
        name="s4_gmlp_fwd_bwd",
    )(u2, do2, B_w_in, B_w_sp, B_w_out.T, mcat,
      A_A_re, A_A_im, A_B_re, A_B_im, A_C_re, A_C_im,
      A_log_dt, A_Dskip, B_b_sp, fm)
    (h2, du, dAr, dAi, dBr, dBi, dCr, dCi, dlog, dD, dwin, dwsp, dbsp, dwout) = outs
    return (h2.T.reshape(1, L, D), du.T.reshape(1, L, D), dAr, dAi, dBr, dBi, dCr, dCi,
            dlog, dD, dwin, dwsp, dbsp, dwout.T)
```

```python
import functools
import numpy as np
import jax
import jax.numpy as jnp
from jax import lax
import jax.experimental.pallas as pl
import jax.experimental.pallas.tpu as pltpu

bf = jnp.bfloat16
f32 = jnp.float32
L = 2048
D = 576
N = 128
T = 128
NC = 16
FH = 2304
EPS = 1e-5
C0 = float(np.sqrt(2.0 / np.pi))
C1 = 0.044715 * C0

NN = (((1,), (0,)), ((), ()))
NT = (((1,), (1,)), ((), ()))
TN = (((0,), (0,)), ((), ()))


def _bf16_round_np(a):
    a = np.ascontiguousarray(np.asarray(a, dtype=np.float32))
    u = a.view(np.uint32).astype(np.uint64)
    r = ((u + 0x7FFF + ((u >> 16) & 1)) >> 16) << 16
    return r.astype(np.uint32).view(np.float32)


def _build_consts():
    lt = _bf16_round_np(np.arange(L)).astype(np.int64)
    bases = []
    for m in range(16):
        step = 1 if m < 2 else 2 if m < 4 else 4 if m < 8 else 8
        for a in range(0, 8, step):
            bases.append(128 * m + a)
    bases.append(2048)
    pos = {}
    valid = set(lt.tolist())
    for i, bs in enumerate(bases):
        t, slot = divmod(i, 8)
        for b in range(16):
            v = bs + 8 * b
            if v in valid:
                assert v not in pos
                pos[v] = (t, 8 * ((b + 1) % 16) + slot)
    assert set(pos.keys()) == valid
    theta = np.pi * (2 * np.arange(T) + 1) / (2 * T)
    tau = np.arange(T)
    Fm = np.concatenate([np.cos(np.outer(tau, theta)), -np.sin(np.outer(tau, theta))], 1)
    Mp = {}
    for m in range(16):
        for l in range(max(0, 128 * m - 127), min(L, 128 * m + 128)):
            r = l - 128 * m
            t, ln = pos[int(lt[l])]
            M = Mp.setdefault((m, t), np.zeros((128, 256)))
            M[ln, :128] += np.cos(theta * r) / T
            M[ln, 128:] += -np.sin(theta * r) / T
    keys = sorted(Mp.keys())
    Mcat = np.concatenate([Mp[k] for k in keys], 0)
    return bases, keys, Mcat.astype(np.float32), Fm.astype(np.float32)


BASES, MKEYS, MCAT_NP, F_NP = _build_consts()
NB = len(BASES)
MIDX = {k: i for i, k in enumerate(MKEYS)}


def _dot(a, b, dims=NN):
    return lax.dot_general(a, b, dims, preferred_element_type=f32)


def _cmul(ar, ai, br, bi):
    return ar * br - ai * bi, ar * bi + ai * br


def _csq(ar, ai):
    return ar * ar - ai * ai, 2.0 * ar * ai


def _gelu_both(x):
    x2 = x * x
    u = x * (C0 + C1 * x2)
    th = jnp.tanh(u)
    hx = 0.5 * x
    s = 1.0 + th
    return hx * s, 0.5 * s + hx * (1.0 - th * th) * (C0 + (3.0 * C1) * x2)


def _gelu(x):
    x2 = x * x
    hx = 0.5 * x
    return hx + hx * jnp.tanh(x * (C0 + C1 * x2))


def _ln0(x):
    m = jnp.sum(x, axis=0, keepdims=True) * (1.0 / D)
    xc = x - m
    v = jnp.sum(xc * xc, axis=0, keepdims=True) * (1.0 / D)
    r = lax.rsqrt(v + EPS)
    return xc * r, r


def _loop(name, n, body, unroll=1):
    assert n % unroll == 0

    def outer(i, c):
        for q in range(unroll):
            body(i * unroll + q, c)
        return c
    with jax.named_scope(name):
        lax.fori_loop(0, n // unroll, outer, 0)


def _steps(m):
    return 1 if m < 2 else 2 if m < 4 else 4 if m < 8 else 8


TICK_P = 1000003
UNR = {"f2": 1, "s4": 2, "s1b": 6, "f3": 4, "s3": 4, "s1a": 2}


def _tick(t):
    return lax.rem(t, jnp.int32(TICK_P))


def kernel(u_hbm, do_hbm, win_hbm, wsp_hbm, wout_hbm, m_hbm,
           Ar_ref, Ai_ref, Br_ref, Bi_ref, Cr_ref, Ci_ref, logdt_ref, dsk_ref, bsp_ref, F_ref,
           h2_hbm, du_hbm, dAr_hbm, dAi_hbm, dBr_hbm, dBi_hbm, dCr_hbm, dCi_hbm, dlog_ref, dD_ref,
           dwin_hbm, dwsp_hbm, dbsp_ref, dwout_hbm,
           U, YH, WIN, WSP, WOUTT, MM, XNT, HT, HNT, DOT_, DHT,
           DZ, XH, KH, PAR, DTC, DSC, BCOL, RS1, RS2, DBROW, R2ROW, MRROW,
           sem_in, sem_h2, sem_du, sem_wsp, sem_win, sem_wout, sem_par):
    BS = 256
    DUT = HT
    DY = YH
    Q1 = DZ.at[:, 0:FH]
    GD2 = DZ.at[:, FH:2 * FH]

    def cin(src, dst, i):
        return pltpu.make_async_copy(src, dst, sem_in.at[i])

    cp_u = cin(u_hbm, U, 0)
    cp_do = cin(do_hbm, DOT_, 1)
    cp_wo8 = cin(wout_hbm.at[:, 8 * 256:FH], WOUTT.at[:, 8 * 256:FH], 2)
    cp_wout = cin(wout_hbm.at[:, 0:8 * 256], WOUTT.at[:, 0:8 * 256], 3)
    cp_m = cin(m_hbm, MM, 4)
    cp_win = cin(win_hbm, WIN, 5)
    cp_wsp = cin(wsp_hbm, WSP, 6)
    for c in (cp_u, cp_do, cp_wo8, cp_wout, cp_m, cp_win, cp_wsp):
        c.start()

    Fm = F_ref[...]

    dt_row = jnp.exp(logdt_ref[...].astype(f32)[None, :]).astype(bf).astype(f32)
    DTC[...] = jnp.broadcast_to(dt_row, (128, D)).T
    DSC[...] = jnp.broadcast_to(dsk_ref[...].astype(f32)[None, :], (128, D)).T
    bsp_row = bsp_ref[...].astype(f32)[None, :]
    for i in range(16):
        BCOL[i * 128:(i + 1) * 128, :] = jnp.broadcast_to(bsp_row[:, i * 128:(i + 1) * 128], (128, 128)).T

    def s0(i, c):
        r = pl.ds(pl.multiple_of(i * 64, 64), 64)
        dt = DTC[r, :]
        ar = dt * Ar_ref[r, :].astype(f32)
        ai = dt * Ai_ref[r, :].astype(f32)
        cbr, cbi = _cmul(Cr_ref[r, :].astype(f32), Ci_ref[r, :].astype(f32),
                         Br_ref[r, :].astype(f32), Bi_ref[r, :].astype(f32))
        PAR[0, r, :] = dt * cbr
        PAR[1, r, :] = dt * cbi
        e = jnp.exp(ar)
        l1 = (e * jnp.cos(ai), e * jnp.sin(ai))
        l2 = _csq(*l1)
        l4 = _csq(*l2)
        l8 = _csq(*l4)
        l128 = _csq(*_csq(*_csq(*_csq(*l8))))
        for k, z in enumerate((l1, l2, l4, l128, l8)):
            PAR[2 + 2 * k, r, :] = z[0]
            PAR[3 + 2 * k, r, :] = z[1]
        return c
    _loop("s0", 9, s0)
    for c in range(8):
        PAR[12, pl.ds(c, 72, stride=8), :] = PAR[10, pl.ds(7 - c, 72, stride=8), :]
        PAR[13, pl.ds(c, 72, stride=8), :] = -PAR[11, pl.ds(7 - c, 72, stride=8), :]

    lane = lax.broadcasted_iota(jnp.int32, (8, 128), 1)
    subl = lax.broadcasted_iota(jnp.int32, (8, 128), 0)
    slot_mask = [(lane & 7) == s for s in range(8)]
    diag_mask = (lane & 7) == subl
    lane8 = ((lane >> 3) * 8).astype(f32)

    def powers16(l8):
        E = [(jnp.ones((8, 128), f32), jnp.zeros((8, 128), f32)), l8]
        for b in range(2, 16):
            E.append(_cmul(*E[-1], *l8))
        return jnp.concatenate(
            [jnp.concatenate([e[0] for e in E], axis=0).astype(bf),
             jnp.concatenate([e[1] for e in E], axis=0).astype(bf)], axis=1)

    def step_ratios(r):
        return {1: (PAR[2, r, :], PAR[3, r, :]), 2: (PAR[4, r, :], PAR[5, r, :]), 4: (PAR[6, r, :], PAR[7, r, :])}

    def gated_lhs(ref, ts, base, ktiles):
        nk = ref.shape[1] // 128
        rows = ref.shape[0]
        gate = dict(zip(ktiles, ts))
        cols = []
        k0 = 0
        for k in sorted(gate) + [nk]:
            if k > k0:
                cols.append(ref[:, k0 * 128:k * 128])
            if k < nk:
                half = rows // 2
                cols.append(jnp.concatenate(
                    [ref[pl.ds(pl.multiple_of((gate[k] - base) * 16 + q * half, 16), half), k * 128:(k + 1) * 128]
                     for q in range(2)], axis=0))
            k0 = k + 1
        return jnp.concatenate(cols, axis=1)

    def ticks(t, n):
        out = []
        for _ in range(n):
            t = _tick(t)
            out.append(t)
        return out

    def rows16(t):
        return pl.ds(pl.multiple_of(t * 16, 16), 16)

    def ssm_fwd(KC, DO, KH32, XH32):
        def dp_cols(rb, col0, ncol):
            rs_ = pl.ds(pl.multiple_of(rb * BS, BS), BS)
            cn = pl.ds(pl.multiple_of(col0, 128), ncol)
            DZ[rs_, cn] = _dot(DO[rs_, :], WOUTT[:, cn]).astype(bf)

        def s1_group(g):
            r = pl.ds(pl.multiple_of(g * 8, 8), 8)
            rhs = powers16((PAR[12, r, :], PAR[13, r, :]))
            lam = step_ratios(r)
            l128 = (PAR[8, r, :], PAR[9, r, :])
            cur = (PAR[0, r, :], PAR[1, r, :])
            Us = []
            for m in range(17):
                z = cur
                if m < 16:
                    st = _steps(m)
                    for a in range(0, 8, st):
                        Us.append(z)
                        if a + st < 8:
                            z = _cmul(*z, *lam[st])
                    cur = _cmul(*cur, *l128)
                else:
                    Us.append(z)
            zero = jnp.zeros((8, 128), f32)
            lhs = jnp.concatenate(
                [jnp.concatenate([x[0] for x in Us] + [zero], axis=0).astype(bf),
                 jnp.concatenate([x[1] for x in Us] + [zero], axis=0).astype(bf)], axis=1)
            out = _dot(lhs, rhs, NT)
            for t in range(6):
                acc = None
                for slot in range(8):
                    i = 8 * t + slot
                    if i >= NB:
                        break
                    rr = pltpu.roll(out[8 * i:8 * i + 8, :], slot + 1, 1, stride=1, stride_axis=0)
                    acc = jnp.where(slot_mask[slot], rr, 0.0 if acc is None else acc)
                KC[r, t * 128:(t + 1) * 128] = acc

        NS1A = 8

        def s1a(i, c):
            for q in range(4):
                s1_group(4 * i + q)
            return c

        _loop("s1a", NS1A, s1a, 4)
        cp_u.wait()
        cp_do.wait()
        cp_wo8.wait()

        def s3(rb, c):
            rs_ = pl.ds(pl.multiple_of(rb * BS, BS), BS)
            dot_ = DOT_[:, rs_].T
            DO[rs_, :] = dot_
            DZ[rs_, 8 * 256:FH] = _dot(dot_, WOUTT[:, 8 * 256:FH]).astype(bf)
            for q in range(2):
                cs = pl.ds(pl.multiple_of(rb * BS + q * 128, 128), 128)
                xn, rs = _ln0(U[:, cs].astype(f32))
                XNT[:, cs] = xn.astype(bf)
                RS1[:, cs] = rs
            return c
        _loop("s3", 8, s3, UNR.get("s3", 1))
        cp_wout.wait()

        def s1b(i, c):
            g0 = 4 * (i + NS1A)
            t0 = 2 * i
            dp_cols(t0 // 16, (t0 % 16) * 128, 128)
            s1_group(g0)
            s1_group(g0 + 1)
            s1_group(g0 + 2)
            s1_group(g0 + 3)
            dp_cols(t0 // 16, (t0 % 16) * 128 + 128, 128)
            return c
        NB1 = 18 - NS1A
        _loop("s1b", NB1, s1b, 5)

        cp_m.wait()
        with jax.named_scope("s2"):
            for m in range(16):
                ts = [t for (mm, t) in MKEYS if mm == m]
                t0 = ts[0]
                i0 = MIDX[(m, t0)]
                nt = len(ts)
                kh = _dot(KC[:, t0 * 128:(t0 + nt) * 128].astype(bf), MM[i0 * 128:(i0 + nt) * 128, :])
                KH32[m] = kh
                KH[m] = kh.astype(bf)
            for j in range(16):
                xh = _dot(XNT[:, j * 128:(j + 1) * 128], Fm)
                XH32[j] = xh
                XH[j] = xh.astype(bf)

        NG4 = 6
        NT4 = 3 * NG4

        def s4(i, c):
            RC = 4
            pts = [(n, cc) for n in range(NT4) for cc in range(RC)][2:-2]
            t0 = NG4 * i
            ts = {}
            t = t0
            for p_ in pts:
                t = _tick(t)
                ts[p_] = t
            blocks = [(q, i0) for q in range(NG4) for i0 in range(14, -1, -2)]
            nsteps = sum(i0 + 2 for _, i0 in blocks)
            cnt = [0]

            def next_t():
                idx = cnt[0] * len(pts) // nsteps
                cnt[0] += 1
                return ts[pts[idx]]

            for q, i0 in blocks:
                acc = {}
                kc = {}
                r = None
                for j in range(i0 + 2):
                    r = rows16(next_t() + q)
                    x = (XH32[j, r, 0:128], XH32[j, r, 128:256])
                    xs = x[0] + x[1]
                    for ii in range(max(i0, j), i0 + 2):
                        m = ii - j
                        if m not in kc:
                            kr, ki = KH32[m, r, 0:128], KH32[m, r, 128:256]
                            kc[m] = (kr, ki, kr + ki)
                        t3 = (kc[m][0] * x[0], kc[m][1] * x[1], kc[m][2] * xs)
                        acc[ii] = tuple(a + b for a, b in zip(acc[ii], t3)) if ii in acc else t3
                for ii in range(i0, i0 + 2):
                    YH[ii, r, 0:128] = (acc[ii][0] - acc[ii][1]).astype(bf)
                    YH[ii, r, 128:256] = (acc[ii][2] - acc[ii][0] - acc[ii][1]).astype(bf)
            rcz = BS // RC
            for n in range(NT4):
                tile = 2 * NB1 + NT4 * i + n
                rb = tile // 16
                rs_ = pl.ds(pl.multiple_of(rb * BS, BS), BS)
                cn = pl.ds(pl.multiple_of((tile % 16) * 128, 128), 128)
                parts = []
                for cc in range(RC):
                    base = rb * BS + cc * rcz
                    if (n, cc) in ts:
                        base = base + (ts[(n, cc)] - t0)
                    parts.append(DO[pl.ds(pl.multiple_of(base, 16), rcz), 0:128])
                lhs = jnp.concatenate([jnp.concatenate(parts, axis=0), DO[rs_, 128:D]], axis=1)
                DZ[rs_, cn] = _dot(lhs, WOUTT[:, cn]).astype(bf)
            return c
        _loop("s4", 36 // NG4, s4)

    pl.run_scoped(ssm_fwd, pltpu.VMEM((D, 768), f32), pltpu.VMEM((L, D), bf),
                  pltpu.VMEM((16, D, 256), f32), pltpu.VMEM((16, D, 256), f32))

    def gmlp_and_bwd(Z1, Z2, DG, DBC):
        def gmlp(T2, WT, R2C, MRC, HN, ACC, DHN):
            def s6(i):
                cs = pl.ds(pl.multiple_of(i * 128, 128), 128)
                y = _dot(YH[i], Fm, NT)
                h = U[:, cs].astype(f32) + y + XNT[:, cs].astype(f32) * DSC[...]
                hn, rs = _ln0(h)
                hb = hn.astype(bf)
                HT[:, cs] = h.astype(bf)
                HNT[:, cs] = hb
                RS2[:, cs] = rs
                HN[cs, :] = hb.T

            with jax.named_scope("s6pro"):
                s6(0)
                s6(1)
            cp_win.wait()

            def p2a(rb, c, with_s6=True):
                rs_ = pl.ds(pl.multiple_of(rb * BS, BS), BS)
                hn = HN[rs_, :]
                for ft in range(9):
                    fs = slice(ft * 256, (ft + 1) * 256)
                    zp = _dot(hn, WIN[:, fs])
                    dgf = Q1[rs_, fs].astype(f32) * _gelu(zp)
                    Z1[rs_, fs] = zp.astype(bf)
                    DG[rs_, fs] = dgf.astype(bf)
                    part = dgf[:, 0:128] + dgf[:, 128:256]
                    if ft == 0:
                        ACC[0] = part
                    else:
                        ACC[0] += part
                db = jnp.sum(ACC[0], axis=1, keepdims=True)
                dbb = jnp.broadcast_to(db, (BS, 128))
                DBC[rs_, :] = dbb
                DBROW[:, rs_] = dbb.T[0:8, :]
                if with_s6:
                    s6(2 * rb + 2)
                for ft in range(9):
                    fs = slice(ft * 256, (ft + 1) * 256)
                    zp = _dot(hn, WIN[:, FH + ft * 256:FH + (ft + 1) * 256])
                    z2 = _gelu(zp)
                    Z2[rs_, fs] = z2.astype(bf)
                    GD2[rs_, fs] = zp.astype(bf)
                    zz = z2 * z2
                    p1 = z2[:, 0:128] + z2[:, 128:256]
                    p2 = zz[:, 0:128] + zz[:, 128:256]
                    if ft == 0:
                        ACC[1] = p1
                        ACC[2] = p2
                    else:
                        ACC[1] += p1
                        ACC[2] += p2
                    if ft == 3 and with_s6:
                        s6(2 * rb + 3)
                mean = jnp.sum(ACC[1], axis=1, keepdims=True) * (1.0 / FH)
                var = jnp.maximum(jnp.sum(ACC[2], axis=1, keepdims=True) * (1.0 / FH) - mean * mean, 0.0)
                r2 = lax.rsqrt(var + EPS)
                r2b = jnp.broadcast_to(r2, (BS, 128))
                mrb = jnp.broadcast_to(mean * r2, (BS, 128))
                R2C[rs_, :] = r2b
                MRC[rs_, :] = mrb
                R2ROW[:, rs_] = r2b.T[0:8, :]
                MRROW[:, rs_] = mrb.T[0:8, :]
                return c
            _loop("p2a", L // BS - 1, p2a)
            with jax.named_scope("p2a_last"):
                p2a(L // BS - 1, 0, with_s6=False)

            cp_wsp.wait()

            def prep_g(rb, offs=(0, 0)):
                n = BS // len(offs)
                for q, off in enumerate(offs):
                    rq = pl.ds(pl.multiple_of(rb * BS + q * n + off * 16, 16), n)
                    wf = WSP[rq, :].astype(f32)
                    WT[q * n:(q + 1) * n, :] = (wf * R2ROW[0:1, :]).astype(bf)
                    ACC[0, q * n:(q + 1) * n, :] = BCOL[rq, :] - jnp.sum(wf * MRROW[0:1, :], axis=1, keepdims=True)

            prep_g(0)

            def p2b(rb, c):
                rs_ = pl.ds(pl.multiple_of(rb * BS, BS), BS)
                wr = WT[...]
                bc = ACC[0][:, 0:1]
                for ft in range(9):
                    fs = slice(ft * 256, (ft + 1) * 256)
                    g = _dot(wr, Z2[:, fs]) + bc
                    z1, gd1 = _gelu_both(Z1[rs_, fs].astype(f32))
                    Z1[rs_, fs] = (z1 * g).astype(bf)
                    Q1[rs_, fs] = (Q1[rs_, fs].astype(f32) * gd1 * g).astype(bf)
                ts = ticks(rb, 4)
                prep_g(jnp.minimum(rb + 1, L // BS - 1), [t - rb for t in ts])
                for q in range(2):
                    rq = pl.ds(pl.multiple_of(rb * BS + q * 128, 128), 128)
                    lhs = gated_lhs(WOUTT, ts, rb, (1, 4, 7, 10)) if q == 0 else WOUTT[...]
                    U[:, rq] = (HT[:, rq].astype(f32) + _dot(lhs, Z1[rq, :], NT)).astype(bf)
                pltpu.make_async_copy(U.at[:, rs_], h2_hbm.at[:, rs_], sem_h2.at[rb]).start()
                return c
            _loop("p2b", L // BS, p2b)

            def prep_t(rb, offs=(0,)):
                n = L // len(offs)
                for q, off in enumerate(offs):
                    WT[:, q * n:(q + 1) * n] = WSP[q * n:(q + 1) * n,
                                                   pl.ds(pl.multiple_of(rb * BS + off * 128, 128), BS)].T

            def fin_dh(rb):
                rs_ = pl.ds(pl.multiple_of(rb * BS, BS), BS)
                dhn = DHN[...]
                hn = HNT[:, rs_].astype(f32)
                a1 = jnp.sum(dhn, axis=0, keepdims=True) * (1.0 / D)
                a2 = jnp.sum(dhn * hn, axis=0, keepdims=True) * (1.0 / D)
                dh = RS2[:, rs_] * (dhn - a1 - hn * a2) + DOT_[:, rs_].astype(f32)
                DHT[:, rs_] = dh.astype(bf)

            def dy_hat(rb):
                for q in range(2):
                    cs = pl.ds(pl.multiple_of(rb * BS + q * 128, 128), 128)
                    DY[2 * rb + q] = _dot(DHT[:, cs], Fm).astype(bf)

            prep_t(0)
            DHN[...] = jnp.zeros((D, BS), f32)
            DHT[:, 0:BS] = jnp.zeros((D, BS), bf)

            def p2c(rb, c):
                rs_ = pl.ds(pl.multiple_of(rb * BS, BS), BS)
                dprev = [DHT[:, pl.ds(pl.multiple_of(jnp.maximum(rb - 2, 0) * BS + q * 128, 128), 128)]
                         for q in range(2)]
                fin_dh(jnp.maximum(rb - 1, 0))
                wt = WT[...]
                s1 = s2 = None
                for ft in range(9):
                    fs = slice(ft * 256, (ft + 1) * 256)
                    dz = _dot(wt, DG[:, fs])
                    T2[:, fs] = dz
                    pz = dz * Z2[rs_, fs].astype(f32)
                    a = dz[:, 0:128] + dz[:, 128:256]
                    b = pz[:, 0:128] + pz[:, 128:256]
                    s1 = a if s1 is None else s1 + a
                    s2 = b if s2 is None else s2 + b
                r2 = R2C[rs_, :][:, 0:1]
                mr = MRC[rs_, :][:, 0:1]
                c1 = jnp.sum(s1, axis=1, keepdims=True) * (1.0 / FH)
                c2 = jnp.sum(s2, axis=1, keepdims=True) * (1.0 / FH) * r2 - c1 * mr
                for ft in range(9):
                    fs = slice(ft * 256, (ft + 1) * 256)
                    z2n = Z2[rs_, fs].astype(f32) * r2 - mr
                    _, gd2 = _gelu_both(GD2[rs_, fs].astype(f32))
                    dz2 = r2 * (T2[:, fs] - c1 - z2n * c2) * gd2
                    GD2[rs_, fs] = dz2.astype(bf)
                ts = ticks(rb, 4)
                prep_t(jnp.minimum(rb + 1, L // BS - 1), [t - rb for t in ts])
                DHN[...] = _dot(gated_lhs(WIN, ts, rb, (20, 23, 26, 29)), DZ[rs_, :], NT)
                for q in range(2):
                    DY[2 * jnp.maximum(rb - 2, 0) + q] = _dot(dprev[q], Fm).astype(bf)
                return c
            _loop("p2c", L // BS, p2c)
            fin_dh(L // BS - 1)
            dy_hat(L // BS - 2)
            dy_hat(L // BS - 1)

        pl.run_scoped(gmlp, pltpu.VMEM((BS, FH), f32), pltpu.VMEM((BS, L), bf), pltpu.VMEM((L, 128), f32),
                      pltpu.VMEM((L, 128), f32), pltpu.VMEM((L, D), bf), pltpu.VMEM((3, BS, 128), f32),
                      pltpu.VMEM((D, BS), f32))

        def ssm_bwd(DXH, DKH, DKC, DDT, DDS, PF, OUTS):
            def ldc(R, m, r):
                return R[m, r, 0:128].astype(f32), R[m, r, 128:256].astype(f32)

            def lda(R, m, r):
                a = ldc(R, m, r)
                return a + (a[0] - a[1],)

            def ldb(R, m, r):
                b = ldc(R, m, r)
                return b + (b[0] + b[1],)

            def mac(acc, key, a, b):
                t = (a[0] * b[0], a[1] * b[1], a[2] * b[2])
                acc[key] = tuple(x + y for x, y in zip(acc[key], t)) if key in acc else t

            def cvt(i, c):
                r = pl.ds(pl.multiple_of(i * 64, 64), 64)
                for k, R in enumerate((Ar_ref, Ai_ref, Br_ref, Bi_ref, Cr_ref, Ci_ref)):
                    PF[k, r, :] = R[r, :].astype(f32)
                return c
            _loop("cvt", 9, cvt)

            NG2 = 4

            def f2(it, c):
                g0 = NG2 * it
                RC = 3
                pts = [(q, n, kq, cc) for q in range(NG2) for n in range(2) for kq in range(4)
                       for cc in range(RC)][1:-1]
                ts = {}
                t = g0
                for p_ in pts:
                    t = _tick(t)
                    ts[p_] = t
                blocks = []
                for q in range(NG2):
                    for i0 in range(0, 16, 2):
                        blocks += [(q, 0, i0), (q, 1, i0)]
                nsteps = sum(16 - i0 for _, _, i0 in blocks)
                cnt = [0]

                def next_t():
                    idx = cnt[0] * len(pts) // nsteps
                    cnt[0] += 1
                    return ts[pts[idx]]

                for q, kind, i0 in blocks:
                    acc = {}
                    cache = {}
                    r = None
                    if kind == 0:
                        for ii in range(i0, 16):
                            r = rows16(next_t() + q)
                            y = ldb(DY, ii, r)
                            for j in range(i0, min(ii, i0 + 1) + 1):
                                m = ii - j
                                if m not in cache:
                                    cache[m] = lda(KH, m, r)
                                mac(acc, j, cache[m], y)
                        dst = DXH
                    else:
                        for j in range(16 - i0):
                            r = rows16(next_t() + q)
                            x = lda(XH, j, r)
                            for m in range(i0, i0 + 2):
                                if j + m > 15:
                                    continue
                                if j + m not in cache:
                                    cache[j + m] = ldb(DY, j + m, r)
                                mac(acc, m, x, cache[j + m])
                        dst = DKH
                    for j in range(i0, i0 + 2):
                        dst[j, r, 0:128] = (acc[j][0] + acc[j][1]).astype(bf)
                        dst[j, r, 128:256] = (acc[j][2] - acc[j][0] + acc[j][1]).astype(bf)
                rcz = 288 // RC
                for q in range(NG2):
                    rh = q % 2
                    ct = (NG2 // 2) * it + q // 2
                    ro = slice(rh * 288, (rh + 1) * 288)
                    for n in range(2):
                        cn = pl.ds(pl.multiple_of(ct * 256 + n * 128, 128), 128)
                        cols = []
                        for kk in range(16):
                            parts = []
                            for cc in range(RC):
                                base = rh * 288 + cc * rcz
                                if kk % 4 == 0 and (q, n, kk // 4, cc) in ts:
                                    parts.append(HNT[pl.ds(pl.multiple_of(base + (ts[(q, n, kk // 4, cc)] - g0), 16),
                                                           rcz), kk * 128:(kk + 1) * 128])
                                else:
                                    parts.append(HNT[base:base + rcz, kk * 128:(kk + 1) * 128])
                            cols.append(jnp.concatenate(parts, axis=0))
                        WIN[ro, cn] = _dot(jnp.concatenate(cols, axis=1), DZ[:, cn]).astype(bf)
                    if rh == 1:
                        co = pl.ds(pl.multiple_of(ct * 256, 256), 256)
                        pltpu.make_async_copy(WIN.at[:, co], dwin_hbm.at[:, co], sem_win.at[ct]).start()
                return c
            _loop("f2", 36 // NG2, f2)

            with jax.named_scope("dkt"):
                for t in range(6):
                    ms = [m for (m, tt) in MKEYS if tt == t]
                    acc = None
                    for m in ms:
                        i0 = MIDX[(m, t)]
                        part = _dot(DKH[m], MM[i0 * 128:(i0 + 1) * 128, :], NT)
                        acc = part if acc is None else acc + part
                    DKC[:, t * 128:(t + 1) * 128] = acc

            def f4_group(g):
                r = pl.ds(pl.multiple_of(g * 8, 8), 8)
                rhs = powers16((PAR[10, r, :], PAR[11, r, :]))
                rows = []
                for i in range(NB):
                    t, slot = divmod(i, 8)
                    rr = pltpu.roll(DKC[r, t * 128:(t + 1) * 128], 120 - slot, 1, stride=1, stride_axis=0)
                    cpl = jnp.where(diag_mask, rr, 0.0)
                    rows.append(cpl)
                    rows.append(cpl * (lane8 + float(BASES[i])))
                lhs = jnp.concatenate(rows, axis=0).astype(bf)
                out = _dot(lhs, rhs)
                lam = step_ratios(r)
                l128 = (PAR[8, r, :], PAR[9, r, :])
                res = []
                for w in range(2):
                    def G(i):
                        return (out[16 * i + 8 * w:16 * i + 8 * w + 8, 0:128],
                                out[16 * i + 8 * w:16 * i + 8 * w + 8, 128:256])
                    S = None
                    idx = NB
                    for m in range(16, -1, -1):
                        nb = 1 if m == 16 else 8 // _steps(m)
                        idx -= nb
                        inner = G(idx + nb - 1)
                        for a in range(nb - 2, -1, -1):
                            pr, pi_ = _cmul(*inner, *lam[_steps(m)])
                            gr, gi = G(idx + a)
                            inner = (pr + gr, pi_ + gi)
                        if S is None:
                            S = inner
                        else:
                            pr, pi_ = _cmul(*S, *l128)
                            S = (pr + inner[0], pi_ + inner[1])
                    res.append(S)
                (s1r, s1i), (s2r, s2i) = res
                gWr, gWi = s1r, -s1i
                dt = DTC[r, :]
                wr, wi = PAR[0, r, :], PAR[1, r, :]
                gar = wr * s2r - wi * s2i
                gai = -(wr * s2i + wi * s2r)
                Arv, Aiv, Brv, Biv, Crv, Civ = [PF[k, r, :] for k in range(6)]
                OUTS[0, r, :] = dt * gar
                OUTS[1, r, :] = dt * gai
                OUTS[2, r, :] = dt * (gWr * Crv + gWi * Civ)
                OUTS[3, r, :] = dt * (gWi * Crv - gWr * Civ)
                OUTS[4, r, :] = dt * (gWr * Brv + gWi * Biv)
                OUTS[5, r, :] = dt * (gWi * Brv - gWr * Biv)
                tot = dt * (gar * Arv + gai * Aiv) + (gWr * wr + gWi * wi)
                DDT[r, :] = jnp.broadcast_to(jnp.sum(tot, axis=1, keepdims=True), (8, 128))

            def f4(rb, c):
                rs_ = pl.ds(pl.multiple_of(rb * BS, BS), BS)
                dgr = DG[rs_, :]
                dbc = DBC[rs_, :][:, 0:1]
                for k in range(9):
                    f4_group(9 * rb + k)
                    if k < 8:
                        ks = slice(k * 256, (k + 1) * 256)
                        a = _dot(dgr, Z2[ks, :], NT)
                        WSP[rs_, ks] = (a * R2ROW[0:1, ks] - dbc * MRROW[0:1, ks]).astype(bf)
                pltpu.make_async_copy(WSP.at[rs_, :], dwsp_hbm.at[rs_, :], sem_wsp.at[rb]).start()
                return c
            _loop("f4", 8, f4, 2)

            for k, R in enumerate((dAr_hbm, dAi_hbm, dBr_hbm, dBi_hbm, dCr_hbm, dCi_hbm)):
                KH[k, :, 0:128] = OUTS[k].astype(bf)
                pltpu.make_async_copy(KH.at[k, :, 0:128], R, sem_par.at[k]).start()
            dlog_ref[...] = DDT[...].T[0, :].astype(bf)
            dbsp_ref[...] = DBROW[0, :].astype(bf)

            def wout_tile(ct):
                cs = pl.ds(pl.multiple_of(ct * 256, 256), 256)
                WOUTT[:, cs] = _dot(DOT_[...], Z1[:, cs]).astype(bf)
                pltpu.make_async_copy(WOUTT.at[:, cs], dwout_hbm.at[:, cs], sem_wout.at[ct]).start()

            def f3(i, c):
                for q in range(2):
                    cs = pl.ds(pl.multiple_of((2 * i + q) * 128, 128), 128)
                    dh = DHT[:, cs].astype(f32)
                    xn = XNT[:, cs].astype(f32)
                    dxn = _dot(DXH[2 * i + q], Fm, NT) + dh * DSC[...]
                    b1 = jnp.sum(dxn, axis=0, keepdims=True) * (1.0 / D)
                    b2 = jnp.sum(dxn * xn, axis=0, keepdims=True) * (1.0 / D)
                    du = dh + RS1[:, cs] * (dxn - b1 - xn * b2)
                    DUT[:, cs] = du.astype(bf)
                    DDS[...] += dh * xn
                    WOUTT[:, cs] = _dot(DOT_[...], Z1[:, cs]).astype(bf)
                c2 = pl.ds(pl.multiple_of(i * 256, 256), 256)
                pltpu.make_async_copy(DUT.at[:, c2], du_hbm.at[:, c2], sem_du.at[i]).start()
                pltpu.make_async_copy(WOUTT.at[:, c2], dwout_hbm.at[:, c2], sem_wout.at[i]).start()
                return c
            DDS[...] = jnp.zeros((D, 128), f32)
            _loop("f3", 8, f3, UNR.get("f3", 1))
            dsk = jnp.sum(DDS[...], axis=1, keepdims=True)
            dD_ref[...] = jnp.broadcast_to(dsk, (D, 128)).T[0, :].astype(bf)
            wout_tile(8)

        pl.run_scoped(ssm_bwd, pltpu.VMEM((16, D, 256), bf), pltpu.VMEM((16, D, 256), bf),
                      pltpu.VMEM((D, 768), f32), pltpu.VMEM((D, 128), f32), pltpu.VMEM((D, 128), f32),
                      pltpu.VMEM((6, D, 128), f32), pltpu.VMEM((6, D, 128), f32))

    pl.run_scoped(gmlp_and_bwd, pltpu.VMEM((L, FH), bf), pltpu.VMEM((L, FH), bf), pltpu.VMEM((L, FH), bf),
                  pltpu.VMEM((L, 128), f32))

    for rb in range(8):
        rs_ = pl.ds(rb * BS, BS)
        pltpu.make_async_copy(U.at[:, rs_], h2_hbm.at[:, rs_], sem_h2.at[rb]).wait()
        pltpu.make_async_copy(WSP.at[rs_, :], dwsp_hbm.at[rs_, :], sem_wsp.at[rb]).wait()
        pltpu.make_async_copy(DUT.at[:, rs_], du_hbm.at[:, rs_], sem_du.at[rb]).wait()
    for ct in range(18):
        co = pl.ds(ct * 256, 256)
        pltpu.make_async_copy(WIN.at[:, co], dwin_hbm.at[:, co], sem_win.at[ct]).wait()
    for ct in range(9):
        cs = pl.ds(ct * 256, 256)
        pltpu.make_async_copy(WOUTT.at[:, cs], dwout_hbm.at[:, cs], sem_wout.at[ct]).wait()
    for k, R in enumerate((dAr_hbm, dAi_hbm, dBr_hbm, dBi_hbm, dCr_hbm, dCi_hbm)):
        pltpu.make_async_copy(KH.at[k, :, 0:128], R, sem_par.at[k]).wait()


@jax.jit
def pallas_sequential_preLN__ssm_conv_s4__mixer_gmlp__prompt_kernel(A_u, A_A_re, A_A_im, A_B_re, A_B_im, A_C_re, A_C_im, A_log_dt, A_Dskip,
        B_x, B_w_in, B_w_sp, B_b_sp, B_w_out, grad_out):
    u2 = A_u.reshape(L, D).T
    do2 = grad_out.reshape(L, D).T
    mcat = jnp.asarray(MCAT_NP, dtype=bf)
    fm = jnp.asarray(F_NP, dtype=bf)
    anyspec = pl.BlockSpec(memory_space=pl.ANY)
    vspec = pl.BlockSpec(memory_space=pltpu.VMEM)
    sds = jax.ShapeDtypeStruct
    out_shape = [sds((D, L), bf), sds((D, L), bf)] + [sds((D, N), bf)] * 6 + [
        sds((D,), bf), sds((D,), bf), sds((D, 2 * FH), bf), sds((L, L), bf), sds((L,), bf), sds((D, FH), bf)]
    out_specs = [anyspec] * 8 + [vspec, vspec, anyspec, anyspec, vspec, anyspec]
    V = pltpu.VMEM
    scratch = [
        V((D, L), bf), V((16, D, 256), bf), V((D, 2 * FH), bf), V((L, L), bf), V((D, FH), bf),
        V((len(MKEYS) * 128, 256), bf),
        V((D, L), bf), V((D, L), bf), V((D, L), bf), V((D, L), bf), V((D, L), bf),
        V((L, 2 * FH), bf), V((16, D, 256), bf), V((16, D, 256), bf),
        V((14, D, 128), f32), V((D, 128), f32), V((D, 128), f32), V((L, 128), f32),
        V((1, L), f32), V((1, L), f32), V((8, L), f32), V((8, L), f32), V((8, L), f32),
    ] + [pltpu.SemaphoreType.DMA((n,)) for n in (8, 8, 8, 8, 18, 9, 6)]
    outs = pl.pallas_call(
        kernel,
        out_shape=out_shape,
        in_specs=[anyspec] * 6 + [vspec] * 10,
        out_specs=out_specs,
        scratch_shapes=scratch,
        compiler_params=pltpu.CompilerParams(vmem_limit_bytes=128 * 2**20),
        name="s4_gmlp_fwd_bwd",
    )(u2, do2, B_w_in, B_w_sp, B_w_out.T, mcat,
      A_A_re, A_A_im, A_B_re, A_B_im, A_C_re, A_C_im,
      A_log_dt, A_Dskip, B_b_sp, fm)
    (h2, du, dAr, dAi, dBr, dBi, dCr, dCi, dlog, dD, dwin, dwsp, dbsp, dwout) = outs
    return (h2.T.reshape(1, L, D), du.T.reshape(1, L, D), dAr, dAi, dBr, dBi, dCr, dCi,
            dlog, dD, dwin, dwsp, dbsp, dwout.T)
```
